```python
import os as _os
_os.environ.setdefault('JAX_PLATFORMS', 'cpu')
import jax
import jax.numpy as jnp

def _softmax(x, axis=-1):
    return jax.nn.softmax(x, axis=axis)

def _gelu(x):
    return jax.nn.gelu(x, approximate=True)

def _silu(x):
    return jax.nn.silu(x)

def _sigmoid(x):
    return jax.nn.sigmoid(x)

def _layernorm(x, axis=-1, eps=1e-05):
    m = jnp.mean(x, axis=axis, keepdims=True)
    v = jnp.var(x, axis=axis, keepdims=True)
    return (x - m) / jnp.sqrt(v + eps)

def _scatter_add(tgt, idx, src, axis=0):
    return tgt.at[idx].add(src)

def _segment_sum(src, seg, n):
    return jax.ops.segment_sum(src, seg, n)

class _Rng:

    def __init__(self, key):
        self._k = key

    def _next(self):
        self._k, sub = jax.random.split(self._k)
        return sub

    def normal(self, shape):
        return jax.random.normal(self._next(), shape, dtype=jnp.bfloat16)

    def randint(self, lo, hi, shape):
        return jax.random.randint(self._next(), shape, lo, hi, dtype=jnp.int32)

    def uniform(self, shape, lo=0.0, hi=1.0):
        return jax.random.uniform(self._next(), shape, jnp.bfloat16, lo, hi)

    def permutation(self, n):
        return jax.random.permutation(self._next(), n)
kernel_name = 'gated_mix__ssm_conv_h3__memory_aug_recurrent_mem_tr__prompt'

def setup_inputs():
    _rng = _Rng(jax.random.key(int.from_bytes(__import__("os").urandom(4), "little")))
    _w = lambda a: (lambda t: t.astype(jnp.bfloat16) if jnp.issubdtype(t.dtype, jnp.floating) else t)(jnp.asarray(a))

    def _A_setup():
        B, S, D = (1, 2048, 1024)
        ks = 4
        return {'q': _w((lambda *s: _rng.normal(s) * 0.05)(B, S, D)), 'k': _w((lambda *s: _rng.normal(s) * 0.4)(B, S, D)), 'v': _w((lambda *s: _rng.normal(s) * 0.4)(B, S, D)), 'shift_k': _w((lambda *s: _rng.normal(s) * 0.4)(D, ks) * 0.5), 'ssm_k': _w((lambda *s: _rng.normal(s) * 0.4)(D, S) * (1.0 / S ** 0.5)), 'ssm_D': _w((lambda *s: _rng.normal(s) * 0.4)(D))}
    _A_in = _A_setup()

    def _B_setup():
        B, S, Dm = (1, 2048, 1024)
        H, Dh = (32, 128)
        M, seg = (8, 32)
        seg = min(seg, S)
        S = S // seg * seg
        return {'x': _w((lambda *s: _rng.normal(s) * 0.05)(B, S, Dm)), 'mem0': _w((lambda *s: _rng.normal(s) * 0.4)(B, M, Dm)), 'Wq': _w((lambda *s: _rng.normal(s) * 3.2)(Dm, H, Dh) * Dm ** (-0.5)), 'Wk': _w((lambda *s: _rng.normal(s) * 3.2)(Dm, H, Dh) * Dm ** (-0.5)), 'Wv': _w((lambda *s: _rng.normal(s) * 0.4)(Dm, H, Dh) * Dm ** (-0.5)), 'Wo': _w((lambda *s: _rng.normal(s) * 0.4)(H, Dh, Dm) * (H * Dh) ** (-0.5)), 'seg_len': seg}
    _B_in = _B_setup()
    return {'A_q': _A_in['q'], 'A_k': _A_in['k'], 'A_v': _A_in['v'], 'A_shift_k': _A_in['shift_k'], 'A_ssm_k': _A_in['ssm_k'], 'A_ssm_D': _A_in['ssm_D'], 'B_x': _B_in['x'], 'B_mem0': _B_in['mem0'], 'B_Wq': _B_in['Wq'], 'B_Wk': _B_in['Wk'], 'B_Wv': _B_in['Wv'], 'B_Wo': _B_in['Wo'], 'B_seg_len': _B_in['seg_len'], 'gate_w': _w((lambda *s: _rng.normal(s) * 0.05)(1024) * 16.0)}

def reference(A_q, A_k, A_v, A_shift_k, A_ssm_k, A_ssm_D, B_x, B_mem0, B_Wq, B_Wk, B_Wv, B_Wo, B_seg_len, gate_w):

    def _A_ref(q, k, v, shift_k, ssm_k, ssm_D):
        B, S, D = q.shape
        ks = shift_k.shape[-1]
        k_pad = jnp.pad(k, ((0, 0), (ks - 1, 0), (0, 0)))
        k_shift = jnp.zeros_like(k)
        for t in range(ks):
            k_shift = k_shift + k_pad[:, t:t + S, :] * shift_k[:, ks - 1 - t][None, None, :]
        kv = k_shift * v
        L = 2 * S
        kv_pad = jnp.pad(kv, ((0, 0), (0, S), (0, 0)))
        kf_pad = jnp.pad(ssm_k, ((0, 0), (0, S)))
        kv_f = (lambda x, axes=(-2, -1): jnp.fft.rfft2(x.astype(jnp.float32), axes=axes))(kv_pad[:, None, :, :], axes=(1, 2))
        kf_f = (lambda x, axes=(-2, -1): jnp.fft.rfft2(x.astype(jnp.float32), axes=axes))(kf_pad[:, None, :], axes=(1, 2))
        kf_f = (lambda x, *d: x.transpose(*d))(kf_f, 1, 2, 0)
        y_f = kv_f * kf_f[None, :, :, :]
        y = (lambda x, s, axes=(-2, -1): jnp.fft.irfft2(x, s=s, axes=axes).astype(jnp.bfloat16))(y_f, (1, L), axes=(1, 2))[:, 0, :S, :]
        y = y + kv * ssm_D[None, None, :]
        return q * y

    def _B_ref(x, mem0, Wq, Wk, Wv, Wo, seg_len):
        B, S, Dm = x.shape
        H, Dh = (Wq.shape[1], Wq.shape[2])
        M = mem0.shape[1]
        scale = Dh ** (-0.5)
        n_seg = S // seg_len
        L = M + seg_len
        idx = jnp.arange(L)
        mask = (idx[:, None] < M) | (idx[:, None] >= idx[None, :])
        mem = mem0
        outs = []
        for s in range(n_seg):
            xs = x[:, s * seg_len:(s + 1) * seg_len, :].copy()
            h = jnp.concatenate([mem, xs], axis=1)
            q = jnp.einsum('btd,dhe->bhte', h, Wq)
            k = jnp.einsum('btd,dhe->bhte', h, Wk)
            v = jnp.einsum('btd,dhe->bhte', h, Wv)
            scores = jnp.einsum('bhqe,bhke->bhqk', q, k) * scale
            scores = jnp.where(mask[None, None], scores, -1000000000.0)
            p = _softmax(scores, axis=-1)
            o = jnp.einsum('bhqk,bhke->bhqe', p, v)
            o = jnp.einsum('bhte,hed->btd', o, Wo)
            mem = o[:, :M, :].copy()
            outs.append(o[:, M:, :])
        return jnp.concatenate(outs, axis=1)
    x = A_q
    g = _sigmoid((x * gate_w).sum(-1, keepdims=True))
    a = _A_ref(x, A_k, A_v, A_shift_k, A_ssm_k, A_ssm_D)
    b = _B_ref(x, B_mem0, B_Wq, B_Wk, B_Wv, B_Wo, B_seg_len)
    return g * a + (1 - g) * b
```

```python
import functools
import math

import jax
import jax.numpy as jnp
from jax import lax
import jax.experimental.pallas as pl
import jax.experimental.pallas.tpu as pltpu

F32 = jnp.float32
BF16 = jnp.bfloat16
U32 = jnp.uint32

S = 2048
D = 1024
H = 32
DH = 128
MEM = 8
SEG = 32
NSEG = S // SEG
TPS = 24
P0 = S - TPS * (NSEG - 1)
RING = 18
PR = 2 * (MEM + SEG)
CB = 128
NB = S // CB
NCH = D // 128
PVLAG = 3


def _kernel(phases,
            x_hbm, k_hbm, v_hbm, h_hbm, wq_hbm, wk_hbm, wv_hbm, wo_hbm,
            shift_ref, dvec_ref, gw_ref, mem0_ref,
            out_hbm,
            x_v, ybuf, out_v, wqkv, wo_v, stage, ring, cbuf, obuf, lhs_q, lhs_o,
            kin, vin, hin, kpad, kvb, ubuf, hbuf, fmat, gmat, bias,
            sem_c, sem_x, sem_w, sem_o, sem_out):
    w_hbms = (wq_hbm, wk_hbm, wv_hbm)

    def conv_copies(c, slot):
        return (
            pltpu.make_async_copy(k_hbm.at[:, pl.ds(c * 128, 128)], kin.at[slot], sem_c.at[slot, 0]),
            pltpu.make_async_copy(v_hbm.at[:, pl.ds(c * 128, 128)], vin.at[slot], sem_c.at[slot, 1]),
            pltpu.make_async_copy(h_hbm.at[pl.ds(c * 128, 128), :], hin.at[slot], sem_c.at[slot, 2]),
        )

    def w_copy(i):
        return pltpu.make_async_copy(
            w_hbms[i // 4].at[:, pl.ds((i % 4) * 8, 8), :], stage.at[i % 4], sem_w.at[i % 4])

    def wo_copy(n):
        return pltpu.make_async_copy(wo_hbm.at[:, pl.ds(n * 128, 128)], wo_v.at[n], sem_o.at[n])

    x_copy = pltpu.make_async_copy(x_hbm, x_v, sem_x.at[0])

    for cp in conv_copies(0, 0):
        cp.start()
    x_copy.start()
    for i in range(4):
        w_copy(i).start()
    for n in range(8):
        wo_copy(n).start()

    r = lax.broadcasted_iota(jnp.int32, (256, 128), 0)
    t = lax.broadcasted_iota(jnp.int32, (256, 128), 1)
    rr = r & 127
    f = jnp.where(rr < 64, 2 * rr, 2 * (rr - 64) + 1)
    n = ((2 * f + 1) * t + jnp.where(r >= 128, 128, 0)) & 511
    fmat[...] = jnp.cos(n.astype(F32) * (2.0 * math.pi / 512.0)).astype(BF16)
    r = lax.broadcasted_iota(jnp.int32, (128, 256), 1)
    t = lax.broadcasted_iota(jnp.int32, (128, 256), 0)
    rr = r & 127
    f = jnp.where(rr < 64, 2 * rr, 2 * (rr - 64) + 1)
    n = ((2 * f + 1) * t + jnp.where(r >= 128, 128, 0)) & 511
    gmat[...] = (jnp.cos(n.astype(F32) * (2.0 * math.pi / 512.0)) * (1.0 / 128.0)).astype(BF16)

    qi = lax.broadcasted_iota(jnp.int32, (PR, PR), 0)
    ki = lax.broadcasted_iota(jnp.int32, (PR, PR), 1)
    qh = qi >= 40
    kh = ki >= 40
    ql = jnp.where(qh, qi - 40, qi)
    kl = jnp.where(kh, ki - 40, ki)
    ok = jnp.logical_and(qh == kh, jnp.logical_or(ql < MEM, ql >= kl))
    bias[...] = jnp.where(ok, 0.0, jnp.where(qh == kh, -1e9, -jnp.inf)).astype(F32)

    kpad[0:8, :] = jnp.zeros((8, 128), F32)
    obuf[0:TPS, :] = jnp.zeros((TPS, H * DH), BF16)

    def conv_body(c, carry):
        slot = c % 2
        for cp in conv_copies(c, slot):
            cp.wait()

        @pl.when(c + 1 < NCH)
        def _():
            for cp in conv_copies(c + 1, 1 - slot):
                cp.start()

        col = pl.multiple_of(c * 128, 128)
        w = shift_ref[:, pl.ds(col, 128)].astype(F32)
        dv = dvec_ref[:, pl.ds(col, 128)].astype(F32)
        kpad[8:8 + S, :] = kin[slot].astype(F32)
        fm = fmat[...]
        for j in range(NB):
            base = 8 + j * CB
            ks = (kpad[base - 3:base - 3 + CB, :] * w[3:4] + kpad[base - 2:base - 2 + CB, :] * w[2:3]
                  + kpad[base - 1:base - 1 + CB, :] * w[1:2] + kpad[base:base + CB, :] * w[0:1])
            kv = (ks * vin[slot, j * CB:(j + 1) * CB, :].astype(F32)).astype(BF16)
            kvb[j * CB:(j + 1) * CB, :] = kv
            ubuf[j] = jnp.dot(fm, kv, preferred_element_type=F32)
        prev = None
        for m in range(NB):
            hm = lax.dot_general(fm, hin[slot, :, m * CB:(m + 1) * CB], (((1,), (1,)), ((), ())),
                                 preferred_element_type=F32)
            if prev is None:
                hbuf[m] = hm
            else:
                hbuf[m, 0:64] = hm[0:64] - prev[128:192]
                hbuf[m, 64:128] = hm[64:128] + prev[192:256]
                hbuf[m, 128:192] = hm[128:192] + prev[0:64]
                hbuf[m, 192:256] = hm[192:256] - prev[64:128]
            prev = hm
        gm = gmat[...]
        for i in range(NB):
            zr_parts, zi_parts = [], []
            for g in range(0, 128, 16):
                zr = None
                for j in range(i + 1):
                    ur = ubuf[j, g:g + 16, :]
                    ui = ubuf[j, 128 + g:128 + g + 16, :]
                    hr = hbuf[i - j, g:g + 16, :]
                    hi = hbuf[i - j, 128 + g:128 + g + 16, :]
                    tr = ur * hr - ui * hi
                    ti = ur * hi + ui * hr
                    if zr is None:
                        zr, zi = tr, ti
                    else:
                        zr, zi = zr + tr, zi + ti
                zr_parts.append(zr.astype(BF16))
                zi_parts.append(zi.astype(BF16))
            z = jnp.concatenate(zr_parts + zi_parts, axis=0)
            y = jnp.dot(gm, z, preferred_element_type=F32)
            y = y + kvb[i * CB:(i + 1) * CB, :].astype(F32) * dv
            ybuf[i * CB:(i + 1) * CB, pl.ds(col, 128)] = y.astype(BF16)
        return carry

    if "conv" in phases:
        lax.fori_loop(0, NCH, conv_body, 0)
    else:
        for cp in conv_copies(0, 0):
            cp.wait()

    x_copy.wait()
    for i in range(12):
        w_copy(i).wait()
        tsel, grp = i // 4, i % 4
        if "pre" in phases:
            for d0 in range(0, D, 128):
                blk = jnp.swapaxes(stage[grp, d0:d0 + 128], 0, 1)
                wqkv[i * 8:(i + 1) * 8, d0 // 2:d0 // 2 + 64, :] = pltpu.bitcast(blk, U32)
        if i + 4 < 12:
            w_copy(i + 4).start()

        def pre_body(hh, carry, i=i, tsel=tsel, grp=grp):
            wj = pltpu.bitcast(wqkv[i * 8 + hh], BF16)
            res = jnp.dot(x_v[0:P0, :], wj, preferred_element_type=F32).astype(BF16)
            ring[i * 8 + hh, 0:P0, :] = res
            return carry
        if "pre" in phases:
            lax.fori_loop(0, 8, pre_body, 0)
    for n in range(8):
        wo_copy(n).wait()

    lhs_q[0:MEM, :] = mem0_ref[...]
    gw = gw_ref[...].astype(F32)
    scale = DH ** -0.5

    def combine(b, rows_start, nrows):
        xt = x_v[pl.ds(rows_start, nrows), :].astype(F32)
        g = jax.nn.sigmoid(jnp.sum(xt * gw, axis=-1, keepdims=True))
        a = xt * ybuf[pl.ds(rows_start, nrows), :].astype(F32)
        out_v[pl.ds(rows_start, nrows), :] = (g * a + (1.0 - g) * b).astype(BF16)

    def step(s, carry):
        p = pl.multiple_of(jnp.minimum(P0 + TPS * s, S - TPS), 8)
        lag = pl.multiple_of(jnp.maximum(TPS * (s - 1), 0), 8)
        lhs_q[MEM:, :] = x_v[pl.ds(p, TPS), :]
        lhs_o[MEM:, :] = obuf[pl.ds(lag, TPS), :]
        lhs = lhs_q[...]
        cur = pl.multiple_of((s % RING) * SEG, SEG)
        offs = [pl.multiple_of((p + 8 * k) % (RING * SEG), 8) for k in range(TPS // 8)]
        for j in range(3 * H):
            cbuf[j // 2, (j % 2) * 40 + MEM:(j % 2) * 40 + 40, :] = ring[j, pl.ds(cur, SEG), :]
        tok0 = pl.multiple_of(s * SEG, SEG)
        def qkv(pr):
            for tsel in range(3):
                for hh in range(2):
                    j = tsel * H + 2 * pr + hh
                    res = jnp.dot(lhs, pltpu.bitcast(wqkv[j], BF16),
                                  preferred_element_type=F32).astype(BF16)
                    cbuf[tsel * 16 + pr, hh * 40:hh * 40 + MEM, :] = res[0:MEM]
                    for k in range(TPS // 8):
                        ring[j, pl.ds(offs[k], 8), :] = res[MEM + 8 * k:MEM + 8 * (k + 1)]

        probs = {}

        def scores(pr):
            qp = cbuf[pr]
            kp = cbuf[16 + pr]
            sc = lax.dot_general(qp, kp, (((1,), (1,)), ((), ())), preferred_element_type=F32) * scale
            fill = bias[...]
            sc = jnp.where(fill == 0.0, sc, fill)
            mx = jnp.max(sc, axis=-1, keepdims=True)
            e = jnp.exp(sc - mx)
            den = jnp.sum(e, axis=-1, keepdims=True)
            rc = pl.reciprocal(den, approx=True)
            rc = rc * (2.0 - den * rc)
            probs[pr] = (e.astype(BF16), rc)

        def pv(pr):
            e, rc = probs.pop(pr)
            vp = cbuf[32 + pr]
            o = (jnp.dot(e, vp, preferred_element_type=F32) * rc).astype(BF16)
            for hh in range(2):
                c0 = (2 * pr + hh) * DH
                lhs_o[0:MEM, c0:c0 + DH] = o[hh * 40:hh * 40 + MEM]
                obuf[pl.ds(tok0, SEG), c0:c0 + DH] = o[hh * 40 + MEM:hh * 40 + 40]

        accs = [None] * (D // 128)

        def wo(pr):
            lo = lhs_o[:, pr * 256:(pr + 1) * 256]
            for nb in range(D // 128):
                t = jnp.dot(lo, wo_v[nb, pr * 256:(pr + 1) * 256, :], preferred_element_type=F32)
                accs[nb] = t if accs[nb] is None else accs[nb] + t

        NP = H // 2
        for pr in range(NP):
            qkv(pr)
            if pr >= 1:
                scores(pr - 1)
            if pr >= PVLAG:
                pv(pr - PVLAG)
        done_pv = NP - PVLAG
        nwo = 0
        first = True
        while nwo < NP:
            for _ in range(3):
                if nwo < NP and nwo < done_pv - (0 if done_pv == NP else 1):
                    wo(nwo)
                    nwo += 1
            if first:
                scores(NP - 1)
                first = False
            if done_pv < NP:
                pv(done_pv)
                done_pv += 1
        acc = jnp.concatenate(accs, axis=1)
        lhs_q[0:MEM, :] = acc[0:MEM].astype(BF16)
        combine(acc[MEM:], lag, TPS)
        return carry

    if "main" in phases:
        lax.fori_loop(0, NSEG, step, 0)

    if "epi" in phases:
        r0 = TPS * (NSEG - 1)
        for (a0, na) in ((r0, 136), (r0 + 136, 128), (r0 + 264, 128), (r0 + 392, 144)):
            lo = obuf[a0:a0 + na, :]
            b = jnp.concatenate(
                [jnp.dot(lo, wo_v[nb], preferred_element_type=F32) for nb in range(D // 128)], axis=1)
            combine(b, a0, na)
    oc = pltpu.make_async_copy(out_v, out_hbm, sem_out.at[0])
    oc.start()
    oc.wait()


def build(phases=("conv", "pre", "main", "epi")):
    @functools.partial(jax.jit, static_argnames=("B_seg_len",))
    def fn(A_q, A_k, A_v, A_shift_k, A_ssm_k, A_ssm_D, B_x, B_mem0, B_Wq, B_Wk, B_Wv, B_Wo,
           B_seg_len, gate_w):
        assert int(B_seg_len) == SEG
        any_spec = pl.BlockSpec(memory_space=pl.ANY)
        vm = pl.BlockSpec(memory_space=pltpu.VMEM)
        out = pl.pallas_call(
            functools.partial(_kernel, phases),
            out_shape=jax.ShapeDtypeStruct((S, D), BF16),
            in_specs=[any_spec] * 8 + [vm] * 4,
            out_specs=any_spec,
            scratch_shapes=[
                pltpu.VMEM((S, D), BF16),
                pltpu.VMEM((S, D), BF16),
                pltpu.VMEM((S, D), BF16),
                pltpu.VMEM((3 * H, D // 2, DH), U32),
                pltpu.VMEM((D // 128, H * DH, 128), BF16),
                pltpu.VMEM((4, D, 8, DH), BF16),
                pltpu.VMEM((3 * H, RING * SEG, DH), BF16),
                pltpu.VMEM((3 * 16, PR, DH), BF16),
                pltpu.VMEM((S, H * DH), BF16),
                pltpu.VMEM((MEM + TPS, D), BF16),
                pltpu.VMEM((MEM + TPS, H * DH), BF16),
                pltpu.VMEM((2, S, 128), BF16),
                pltpu.VMEM((2, S, 128), BF16),
                pltpu.VMEM((2, 128, S), BF16),
                pltpu.VMEM((S + 8, 128), F32),
                pltpu.VMEM((S, 128), BF16),
                pltpu.VMEM((NB, 256, 128), F32),
                pltpu.VMEM((NB, 256, 128), F32),
                pltpu.VMEM((256, 128), BF16),
                pltpu.VMEM((128, 256), BF16),
                pltpu.VMEM((PR, PR), F32),
                pltpu.SemaphoreType.DMA((2, 3)),
                pltpu.SemaphoreType.DMA((1,)),
                pltpu.SemaphoreType.DMA((4,)),
                pltpu.SemaphoreType.DMA((8,)),
                pltpu.SemaphoreType.DMA((1,)),
            ],
            compiler_params=pltpu.CompilerParams(vmem_limit_bytes=120 * 1024 * 1024),
        )(A_q.reshape(S, D), A_k.reshape(S, D), A_v.reshape(S, D), A_ssm_k,
          B_Wq, B_Wk, B_Wv, B_Wo.reshape(H * DH, D),
          A_shift_k.T, A_ssm_D.reshape(1, D), gate_w.reshape(1, D), B_mem0.reshape(MEM, D))
        return out.reshape(1, S, D)
    return fn


pallas_gated_mix__ssm_conv_h3__memory_aug_recurrent_mem_tr__prompt_kernel = build()
```

```python
import functools
import math

import jax
import jax.numpy as jnp
from jax import lax
import jax.experimental.pallas as pl
import jax.experimental.pallas.tpu as pltpu

F32 = jnp.float32
BF16 = jnp.bfloat16
U32 = jnp.uint32

S = 2048
D = 1024
H = 32
DH = 128
MEM = 8
SEG = 32
NSEG = S // SEG
TPS = 24
P0 = S - TPS * (NSEG - 1)
PM = 544
RING = 18
PR = 2 * (MEM + SEG)
CB = 128
NB = S // CB
NCH = D // 128
PVLAG = 3
NSLOT = 3
NCHUNK = 6
PPA = 4
PPI = 5
RG = 8
SIDE = (('k', 0), ('k', 1), ('k', 2), ('r', 1), ('k', 3), ('r', 2), ('r', 3), ('r', 4))
U_AFTER = (2, 3, 5, 6)
KG = 8
GR = 16
MSUB = ((0, 144), (144, 144), (288, 128), (416, 128))
INV_AFTER = {11: (0, 1), 13: (2, 3), 15: (4, 5), 18: (6, 7), 22: (8, 9), 27: (10, 11), 32: (12, 13), 38: (14, 15)}
KV0 = 2 * PPI * (D // 2)
OCH = 192
EPI = ((1512, 136), (1648, 128), (1776, 128), (1904, 144))


def _kernel(phases,
            x_hbm, k_hbm, v_hbm, h_hbm, wq_hbm, wk_hbm, wv_hbm, wo_hbm,
            shift_ref, dvec_ref, gw_ref, mem0_ref,
            out_hbm,
            x_v, x0, ybuf, out_v, wqkv, wt0, wt1, wt2, wt3, wt4, kv0, kv1, kv2, kv3, wo_v, stage, ring, cbuf, obuf, lhs_q, lhs_o,
            kin, vin, hin, kpad, spec, fmat, gmat, bias, zsm,
            sem_c, sem_x, sem_w, sem_o, sem_out):
    w_u32 = tuple(w.bitcast(U32) for w in (wq_hbm, wk_hbm, wv_hbm))
    wo_u32 = wo_hbm.bitcast(U32)
    stage4 = stage.reshape(NSLOT * 2, D // 2, 8, DH)
    wtmp = (wt0, wt1, wt2, wt3, wt4)
    kvb = (kv0, kv1, kv2, kv3)

    def conv_copies(c, slot):
        return (
            pltpu.make_async_copy(k_hbm.at[:, pl.ds(c * 128, 128)], kin.at[slot], sem_c.at[slot, 0]),
            pltpu.make_async_copy(v_hbm.at[:, pl.ds(c * 128, 128)], vin.at[slot], sem_c.at[slot, 1]),
            pltpu.make_async_copy(h_hbm.at[pl.ds(c * 128, 128), :], hin.at[slot], sem_c.at[slot, 2]),
        )

    class w_copy:
        def __init__(self, i, quarter=None):
            r0, nr, s0 = (0, 8, 0) if quarter is None else (4 * quarter, 4, 2 * quarter)
            self.cps = [pltpu.make_async_copy(
                w_u32[i // 2].at[:, par, pl.ds((i % 2) * 8 + r0, nr), :],
                stage4.at[2 * (i % NSLOT) + par, :, pl.ds(r0, nr), :],
                sem_w.at[i % NSLOT, s0 + par]) for par in range(2)]

        def start(self):
            for cp in self.cps:
                cp.start()

        def wait(self):
            for cp in self.cps:
                cp.wait()

    def wo_copy(n):
        return pltpu.make_async_copy(wo_u32.at[:, pl.ds(n * 128, 128)], wo_v.at[n], sem_o.at[n])

    def x_copy(half):
        rows = pl.ds(half * (S // 2), S // 2)
        return pltpu.make_async_copy(x_hbm.at[rows, :], x_v.at[rows, :], sem_x.at[1 + half])

    def out_copy(r0, nr, k):
        return pltpu.make_async_copy(out_v.at[pl.ds(r0, nr), :], out_hbm.at[pl.ds(r0, nr), :], sem_out.at[k])

    x0_copy = pltpu.make_async_copy(x_hbm.bitcast(U32).at[pl.ds(0, PM // 2), :], x0, sem_x.at[0])
    x0_copy.start()
    w_copy(0, 0).start()

    r = lax.broadcasted_iota(jnp.int32, (256, 128), 0)
    t = lax.broadcasted_iota(jnp.int32, (256, 128), 1)
    rr = r & 127
    f = jnp.where(rr < 64, 2 * rr, 2 * (rr - 64) + 1)
    n = ((2 * f + 1) * t + jnp.where(r >= 128, 128, 0)) & 511
    fmat[...] = jnp.cos(n.astype(F32) * (2.0 * math.pi / 512.0)).astype(BF16)
    r = lax.broadcasted_iota(jnp.int32, (128, 256), 1)
    t = lax.broadcasted_iota(jnp.int32, (128, 256), 0)
    rr = r & 127
    f = jnp.where(rr < 64, 2 * rr, 2 * (rr - 64) + 1)
    n = ((2 * f + 1) * t + jnp.where(r >= 128, 128, 0)) & 511
    gmat[...] = (jnp.cos(n.astype(F32) * (2.0 * math.pi / 512.0)) * (1.0 / 128.0)).astype(BF16)

    qi = lax.broadcasted_iota(jnp.int32, (PR, PR), 0)
    ki = lax.broadcasted_iota(jnp.int32, (PR, PR), 1)
    qh = qi >= 40
    kh = ki >= 40
    ql = jnp.where(qh, qi - 40, qi)
    kl = jnp.where(kh, ki - 40, ki)
    ok = jnp.logical_and(qh == kh, jnp.logical_or(ql < MEM, ql >= kl))
    bias[...] = jnp.where(ok, 0.0, jnp.where(qh == kh, -1e9, -jnp.inf)).astype(F32)

    zsm[0] = 0
    kpad[0:8, :] = jnp.zeros((8, 128), F32)
    obuf[0:TPS, :] = jnp.zeros((TPS, H * DH), BF16)

    def relayout(q, k, zero, always, m, dbl):
        base = ((q // 8) % NSLOT) * (D * 8) + q % 8
        low = jnp.full((RG, DH), 0xFFFF, U32)
        high = jnp.full((RG, DH), 0xFFFF0000, U32)
        m = low if m is None else jnp.where(always, low, m)
        for r0 in range(0, D // 2, RG):
            a = stage[pl.ds(base + r0 * 8, RG, stride=8), :]
            b = stage[pl.ds(base + D * 4 + r0 * 8, RG, stride=8), :]
            lo = (a & m) | (b << 16)
            if always is not None:
                hi = (a >> 16) | (b & (jnp.where(always, high, lo) if dbl else high))
                m = jnp.where(always, low, hi if dbl else lo)
            else:
                hi = (a >> 16) | (b & high)
            wtmp[k][zero, r0:r0 + RG, :] = lo
            wtmp[k][zero + 1, r0:r0 + RG, :] = hi
            wqkv[2 * q, r0:r0 + RG, :] = lo
            wqkv[2 * q + 1, r0:r0 + RG, :] = hi
        return m

    def proj(q0, su, zero):
        j = 2 * q0 + su // 4
        r0, nr = MSUB[su % 4]
        wj = pltpu.bitcast(wtmp[su // 8][(su // 4) % 2], BF16)
        res = jnp.dot(pltpu.bitcast(x0[r0 // 2:(r0 + nr) // 2, :], BF16), wj,
                      preferred_element_type=F32)
        ring[j, r0:r0 + nr, :] = res.astype(BF16)

    x0_copy.wait()
    w_copy(0, 0).wait()
    w_copy(0, 1).start()
    w_copy(1).start()

    def pro_a(c, carry):
        @pl.when(c == 1)
        def _():
            w_copy(0, 1).wait()
            for cp in conv_copies(0, 0):
                cp.start()
        zero = zsm[0]
        always = jnp.full((8, 128), zero, jnp.int32) == 0
        q0 = c * PPA
        relayout(q0, 0, zero, None, None, False)
        for su in range(8 * PPA):
            proj(q0, su, zero)
            if su % 8 == 0 and su // 8 + 1 < PPA:
                relayout(q0 + su // 8 + 1, su // 8 + 1, zero, always, None, True)
        return carry

    if "pre" in phases:
        lax.fori_loop(0, 8 // PPA, pro_a, 0)
    else:
        w_copy(0, 1).wait()
        for cp in conv_copies(0, 0):
            cp.start()

    W_WAIT = {1: 0, 2: 1, 3: 3, 4: 4, 5: 6}
    W_START = {2: 0, 3: 1, 4: 2, 5: 4}
    for i in range(1, NCHUNK):
        assert W_WAIT[i] == min(c for c in range(NCH) if (8 + PPI * c + PPI - 1) // 8 >= i)
    for i, c0 in W_START.items():
        assert c0 < W_WAIT[i]
        assert all((8 + PPI * c) // 8 > i - NSLOT for c in range(c0, NCH))

    def pro_b(c, carry):
        slot = c % 2
        for i, cw in W_WAIT.items():
            @pl.when(c == cw)
            def _(i=i):
                w_copy(i).wait()
        for cp in conv_copies(c, slot):
            cp.wait()

        @pl.when(c + 1 < NCH)
        def _():
            for cp in conv_copies(c + 1, 1 - slot):
                cp.start()
        for i, cs in W_START.items():
            @pl.when(c == cs)
            def _(i=i):
                w_copy(i).start()
        for cs, n0 in ((3, 0), (5, 4)):
            @pl.when(c == cs)
            def _(n0=n0):
                for n in range(n0, n0 + 4):
                    wo_copy(n).start()

        @pl.when(c == 6)
        def _():
            for half in range(2):
                x_copy(half).start()

        zero = zsm[0]
        always = jnp.full((8, 128), zero, jnp.int32) == 0
        zrow = pl.multiple_of(zero * 16, 16)
        col = pl.multiple_of(c * 128, 128)
        w = shift_ref[:, pl.ds(col, 128)].astype(F32)
        dv = dvec_ref[:, pl.ds(col, 128)].astype(F32)
        q0 = 8 + c * PPI

        w3 = jnp.broadcast_to(w[3:4], (KG, 128))
        pace = [w3]
        gate = [None]

        def kv_mul(j):
            if gate[0] is not None:
                pace[0] = jnp.where(always, w3, pltpu.bitcast(gate[0], F32))
            for r0 in range(j * CB, (j + 1) * CB, 2 * KG):
                kpad[8 + r0:8 + r0 + 2 * KG, :] = kin[slot, r0:r0 + 2 * KG, :].astype(F32)
                vf = vin[slot, r0:r0 + 2 * KG, :].astype(F32)
                kvs = []
                for hf in range(2):
                    base = 8 + r0 + hf * KG
                    ks = (kpad[base - 3:base - 3 + KG, :] * pace[0] + kpad[base - 2:base - 2 + KG, :] * w[2:3]
                          + kpad[base - 1:base - 1 + KG, :] * w[1:2] + kpad[base:base + KG, :] * w[0:1])
                    kv = ks * vf[hf * KG:(hf + 1) * KG]
                    if hf == 1:
                        pace[0] = jnp.where(always, w3, kv)
                    kvs.append(kv)
                rr0 = r0 % (4 * CB)
                kvb[j // 4][pl.ds(zrow + rr0, 2 * KG), :] = jnp.concatenate(kvs, axis=0).astype(BF16)
            gate[0] = pltpu.bitcast(pace[0], U32)

        def kv_load(j):
            return kvb[j // 4][(j % 4) * CB:(j % 4 + 1) * CB, :]

        def u_dft(j):
            spec[zero + j] = jnp.dot(fmat[...], kv_load(j), preferred_element_type=F32)

        def h_dft():
            for m in range(NB):
                spec[zero + NB + m] = lax.dot_general(fmat[...], hin[slot, :, m * CB:(m + 1) * CB],
                                               (((1,), (1,)), ((), ())), preferred_element_type=F32)

        def ld(idx, r0):
            return spec[idx, r0:r0 + GR, :]

        def freq_mul(i):
            for g in range(0, 128, GR):
                sgn = 1.0 if g < 64 else -1.0
                hr1, hi1 = ld(NB + i + 1, g), ld(NB + i + 1, 128 + g)
                if gate[0] is not None:
                    gt = pltpu.bitcast(gate[0], F32)
                    hr1 = jnp.concatenate([jnp.where(always, hr1[0:8], gt), hr1[8:]], axis=0)
                    gate[0] = None
                y0r = y0i = y1r = y1i = None
                for j in range(i + 2):
                    ur, ui = ld(j, g), ld(j, 128 + g)
                    tr = ur * hr1 - ui * hi1
                    ti = ur * hi1 + ui * hr1
                    y1r, y1i = (tr, ti) if y1r is None else (y1r + tr, y1i + ti)
                    if j <= i:
                        hr1, hi1 = ld(NB + i - j, g), ld(NB + i - j, 128 + g)
                        tr = ur * hr1 - ui * hi1
                        ti = ur * hi1 + ui * hr1
                        y0r, y0i = (tr, ti) if y0r is None else (y0r + tr, y0i + ti)
                if sgn > 0:
                    z1r, z1i = y1r - y0i, y1i + y0r
                else:
                    z1r, z1i = y1r + y0i, y1i - y0r
                if i > 0:
                    pr_, pi_ = ld(2 * NB, g), ld(2 * NB, 128 + g)
                    if sgn > 0:
                        y0r, y0i = y0r - pi_, y0i + pr_
                    else:
                        y0r, y0i = y0r + pi_, y0i - pr_
                if i + 2 < NB:
                    spec[zero + 2 * NB, g:g + GR, :] = y1r
                    spec[zero + 2 * NB, 128 + g:128 + g + GR, :] = y1i
                zi = zero + 2 * NB + 1 + i // 2
                h2 = GR // 2
                spec[zi, g // 2:g // 2 + h2, :] = pltpu.bitcast(y0r.astype(BF16), F32)
                spec[zi, 64 + g // 2:64 + g // 2 + h2, :] = pltpu.bitcast(y0i.astype(BF16), F32)
                spec[zi, 128 + g // 2:128 + g // 2 + h2, :] = pltpu.bitcast(z1r.astype(BF16), F32)
                spec[zi, 192 + g // 2:192 + g // 2 + h2, :] = pltpu.bitcast(z1i.astype(BF16), F32)

        def inv(i):
            r0 = (i % 2) * 128
            z = pltpu.bitcast(spec[2 * NB + 1 + i // 2, r0:r0 + 128, :], BF16)
            y = jnp.dot(gmat[...], z, preferred_element_type=F32)
            y = y + kv_load(i).astype(F32) * dv
            ybuf[i * CB:(i + 1) * CB, pl.ds(col, 128)] = y.astype(BF16)

        do_c = "conv" in phases
        do_p = "pre" in phases
        def side(tok):
            if tok[0] == "k" and do_c:
                for j in range(4 * tok[1], 4 * tok[1] + 4):
                    kv_mul(j)
            if tok[0] == "r" and do_p:
                gate[0] = relayout(q0 + tok[1], tok[1], zero, always, gate[0], False)

        if do_p:
            relayout(q0, 0, zero, None, None, False)
        if do_c:
            h_dft()
        for tok in SIDE:
            side(tok)
        for su in range(8 * PPI):
            if do_p:
                proj(q0, su, zero)
            if do_c:
                if su in U_AFTER:
                    for j in range(U_AFTER.index(su) * 4, U_AFTER.index(su) * 4 + 4):
                        u_dft(j)
                for i in INV_AFTER.get(su + 1, ())[:1]:
                    freq_mul(i)
                for i in INV_AFTER.get(su, ()):
                    inv(i)
        return carry

    lax.fori_loop(0, NCH, pro_b, 0)
    for half in range(2):
        x_copy(half).wait()
    for n in range(8):
        wo_copy(n).wait()

    lhs_q[0:MEM, :] = mem0_ref[...]
    gw = gw_ref[...].astype(F32)
    scale = DH ** -0.5

    def combine(b, rows_start, nrows):
        xt = x_v[pl.ds(rows_start, nrows), :].astype(F32)
        g = jax.nn.sigmoid(jnp.sum(xt * gw, axis=-1, keepdims=True))
        a = xt * ybuf[pl.ds(rows_start, nrows), :].astype(F32)
        out_v[pl.ds(rows_start, nrows), :] = (g * a + (1.0 - g) * b).astype(BF16)

    def step(s, carry):
        @pl.when(jnp.logical_and(s % 8 == 1, s > 8))
        def _():
            k = s // 8 - 1
            out_copy(pl.multiple_of(k * OCH, OCH), OCH, k).start()

        p = pl.multiple_of(jnp.minimum(P0 + TPS * s, S - TPS), 8)
        lag = pl.multiple_of(jnp.maximum(TPS * (s - 1), 0), 8)
        lhs_q[MEM:, :] = x_v[pl.ds(p, TPS), :]
        lhs_o[MEM:, :] = obuf[pl.ds(lag, TPS), :]
        lhs = lhs_q[...]
        cur = pl.multiple_of((s % RING) * SEG, SEG)
        offs = [pl.multiple_of((p + 8 * k) % (RING * SEG), 8) for k in range(TPS // 8)]
        for j in range(3 * H):
            cbuf[j // 2, (j % 2) * 40 + MEM:(j % 2) * 40 + 40, :] = ring[j, pl.ds(cur, SEG), :]
        tok0 = pl.multiple_of(s * SEG, SEG)

        def qkv(pr):
            for tsel in range(3):
                for hh in range(2):
                    j = tsel * H + 2 * pr + hh
                    res = jnp.dot(lhs, pltpu.bitcast(wqkv[j], BF16),
                                  preferred_element_type=F32).astype(BF16)
                    cbuf[tsel * 16 + pr, hh * 40:hh * 40 + MEM, :] = res[0:MEM]
                    for k in range(TPS // 8):
                        ring[j, pl.ds(offs[k], 8), :] = res[MEM + 8 * k:MEM + 8 * (k + 1)]

        probs = {}

        def scores(pr):
            qp = cbuf[pr]
            kp = cbuf[16 + pr]
            sc = lax.dot_general(qp, kp, (((1,), (1,)), ((), ())), preferred_element_type=F32) * scale
            fill = bias[...]
            sc = jnp.where(fill == 0.0, sc, fill)
            mx = jnp.max(sc, axis=-1, keepdims=True)
            e = jnp.exp(sc - mx)
            den = jnp.sum(e, axis=-1, keepdims=True)
            rc = pl.reciprocal(den, approx=True)
            rc = rc * (2.0 - den * rc)
            probs[pr] = (e * rc).astype(BF16)

        def pv(pr):
            e = probs.pop(pr)
            vp = cbuf[32 + pr]
            o = jnp.dot(e, vp, preferred_element_type=F32).astype(BF16)
            for hh in range(2):
                c0 = (2 * pr + hh) * DH
                lhs_o[0:MEM, c0:c0 + DH] = o[hh * 40:hh * 40 + MEM]
                obuf[pl.ds(tok0, SEG), c0:c0 + DH] = o[hh * 40 + MEM:hh * 40 + 40]

        accs = [None] * (D // 128)

        def wo(pr):
            lo = lhs_o[:, pr * 256:(pr + 1) * 256]
            for nb in range(D // 128):
                wt = pltpu.bitcast(wo_v[nb, pr * 128:(pr + 1) * 128, :], BF16)
                t = jnp.dot(lo, wt, preferred_element_type=F32)
                accs[nb] = t if accs[nb] is None else accs[nb] + t

        NP = H // 2
        for pr in range(NP):
            qkv(pr)
            if pr >= 1:
                scores(pr - 1)
            if pr >= PVLAG:
                pv(pr - PVLAG)
        done_pv = NP - PVLAG
        nwo = 0
        first = True
        while nwo < NP:
            for _ in range(3):
                if nwo < NP and nwo < done_pv - (0 if done_pv == NP else 1):
                    wo(nwo)
                    nwo += 1
            if first:
                scores(NP - 1)
                first = False
            if done_pv < NP:
                pv(done_pv)
                done_pv += 1
        acc = jnp.concatenate(accs, axis=1)
        lhs_q[0:MEM, :] = acc[0:MEM].astype(BF16)
        combine(acc[MEM:], lag, TPS)
        return carry

    nstream = (NSEG - 1) // 8
    if "main" in phases:
        lax.fori_loop(0, NSEG, step, 0)
    else:
        if "main1" in phases:
            lax.fori_loop(0, 1 + zsm[0], step, 0)
        for k in range(nstream):
            out_copy(k * OCH, OCH, k).start()
    tail0 = nstream * OCH
    out_copy(tail0, EPI[0][0] - tail0, nstream).start()

    for e, (a0, na) in enumerate(EPI):
        if "epi" in phases:
            lo = obuf[a0:a0 + na, :]
            b = jnp.concatenate(
                [jnp.dot(lo, pltpu.bitcast(wo_v[nb], BF16), preferred_element_type=F32)
                 for nb in range(D // 128)], axis=1)
            combine(b, a0, na)
        out_copy(a0, na, nstream + 1 + e).start()
    for k in range(nstream):
        out_copy(k * OCH, OCH, k).wait()
    out_copy(tail0, EPI[0][0] - tail0, nstream).wait()
    for e, (a0, na) in enumerate(EPI):
        out_copy(a0, na, nstream + 1 + e).wait()


def build(phases=("conv", "pre", "main", "epi")):
    @functools.partial(jax.jit, static_argnames=("B_seg_len",))
    def fn(A_q, A_k, A_v, A_shift_k, A_ssm_k, A_ssm_D, B_x, B_mem0, B_Wq, B_Wk, B_Wv, B_Wo,
           B_seg_len, gate_w):
        assert int(B_seg_len) == SEG
        any_spec = pl.BlockSpec(memory_space=pl.ANY)
        vm = pl.BlockSpec(memory_space=pltpu.VMEM)
        out = pl.pallas_call(
            functools.partial(_kernel, phases),
            out_shape=jax.ShapeDtypeStruct((S, D), BF16),
            in_specs=[any_spec] * 8 + [vm] * 4,
            out_specs=any_spec,
            scratch_shapes=[
                pltpu.VMEM((S, D), BF16),
                pltpu.VMEM((PM // 2, D), U32),
                pltpu.VMEM((S, D), BF16),
                pltpu.VMEM((S, D), BF16),
                pltpu.VMEM((3 * H, D // 2, DH), U32),
                pltpu.VMEM((2, D // 2, DH), U32),
                pltpu.VMEM((2, D // 2, DH), U32),
                pltpu.VMEM((2, D // 2, DH), U32),
                pltpu.VMEM((2, D // 2, DH), U32),
                pltpu.VMEM((2, D // 2, DH), U32),
                pltpu.VMEM((S // 4, 128), BF16),
                pltpu.VMEM((S // 4, 128), BF16),
                pltpu.VMEM((S // 4, 128), BF16),
                pltpu.VMEM((S // 4, 128), BF16),
                pltpu.VMEM((D // 128, H * DH // 2, 128), U32),
                pltpu.VMEM((NSLOT * D * 8, DH), U32),
                pltpu.VMEM((3 * H, RING * SEG, DH), BF16),
                pltpu.VMEM((3 * 16, PR, DH), BF16),
                pltpu.VMEM((S, H * DH), BF16),
                pltpu.VMEM((MEM + TPS, D), BF16),
                pltpu.VMEM((MEM + TPS, H * DH), BF16),
                pltpu.VMEM((2, S, 128), BF16),
                pltpu.VMEM((2, S, 128), BF16),
                pltpu.VMEM((2, 128, S), BF16),
                pltpu.VMEM((S + 8, 128), F32),
                pltpu.VMEM((2 * NB + 1 + NB // 2, 256, 128), F32),
                pltpu.VMEM((256, 128), BF16),
                pltpu.VMEM((128, 256), BF16),
                pltpu.VMEM((PR, PR), F32),
                pltpu.SMEM((1,), jnp.int32),
                pltpu.SemaphoreType.DMA((2, 3)),
                pltpu.SemaphoreType.DMA((3,)),
                pltpu.SemaphoreType.DMA((NSLOT, 4)),
                pltpu.SemaphoreType.DMA((8,)),
                pltpu.SemaphoreType.DMA((12,)),
            ],
            compiler_params=pltpu.CompilerParams(vmem_limit_bytes=120 * 1024 * 1024),
        )(A_q.reshape(S, D), A_k.reshape(S, D), A_v.reshape(S, D), A_ssm_k,
          B_Wq.reshape(D // 2, 2, H, DH), B_Wk.reshape(D // 2, 2, H, DH), B_Wv.reshape(D // 2, 2, H, DH),
          B_Wo.reshape(H * DH, D),
          A_shift_k.T, A_ssm_D.reshape(1, D), gate_w.reshape(1, D), B_mem0.reshape(MEM, D))
        return out.reshape(1, S, D)
    return fn


pallas_gated_mix__ssm_conv_h3__memory_aug_recurrent_mem_tr__prompt_kernel = build()
```

```python
import functools
import math

import jax
import jax.numpy as jnp
from jax import lax
import jax.experimental.pallas as pl
import jax.experimental.pallas.tpu as pltpu

F32 = jnp.float32
BF16 = jnp.bfloat16
U32 = jnp.uint32

S = 2048
D = 1024
H = 32
DH = 128
MEM = 8
SEG = 32
NSEG = S // SEG
TPS = 24
P0 = S - TPS * (NSEG - 1)
PM = 544
RING = 18
PR = 2 * (MEM + SEG)
CB = 128
NB = S // CB
NCH = D // 128
DS = 7
DPV = 9
RMODE = 'xor'
KVLINK = 2
GATEZ = False
UNROLL = 2
NDEFER = 5
GATEPR = 2
GROUP = 1
SFIRST = False
OTRIG = UNROLL % 8
NSLOT = 3
NCHUNK = 6
PPA = 4
PPI = 5
RG = 8
SIDE = (('k', 0), ('k', 1), ('k', 2), ('r', 1), ('k', 3), ('r', 2), ('r', 3), ('r', 4))
U_AFTER = (2, 3, 5, 6)
KG = 8
GR = 16
MSUB = (((0, 144),), ((144, 144),), ((288, 128),), ((416, 128),))
INV_AFTER = {11: (0, 1), 13: (2, 3), 15: (4, 5), 18: (6, 7), 22: (8, 9), 27: (10, 11), 32: (12, 13), 38: (14, 15)}
KV0 = 2 * PPI * (D // 2)
OCH = 192
EPI = ((1512, 136), (1648, 128), (1776, 128), (1904, 144))


def _kernel(phases,
            x_hbm, k_hbm, v_hbm, h_hbm, wq_hbm, wk_hbm, wv_hbm, wo_hbm,
            shift_ref, dvec_ref, gw_ref, mem0_ref,
            out_hbm,
            x_v, x0, ybuf, out_v, wqkv, wt0, wt1, wt2, wt3, wt4, kv0, kv1, kv2, kv3, wo_v, stage, ring, cbuf, obuf, lhs_q, lhs_o,
            kin, vin, hin, kpad, spec, fmat, gmat, bias, prm, zsm,
            sem_c, sem_x, sem_w, sem_o, sem_out):
    w_u32 = tuple(w.bitcast(U32) for w in (wq_hbm, wk_hbm, wv_hbm))
    wo_u32 = wo_hbm.bitcast(U32)
    stage4 = stage.reshape(NSLOT * 2, D // 2, 8, DH)
    wtmp = (wt0, wt1, wt2, wt3, wt4)
    kvb = (kv0, kv1, kv2, kv3)

    def conv_copies(c, slot):
        return (
            pltpu.make_async_copy(k_hbm.at[:, pl.ds(c * 128, 128)], kin.at[slot], sem_c.at[slot, 0]),
            pltpu.make_async_copy(v_hbm.at[:, pl.ds(c * 128, 128)], vin.at[slot], sem_c.at[slot, 1]),
            pltpu.make_async_copy(h_hbm.at[pl.ds(c * 128, 128), :], hin.at[slot], sem_c.at[slot, 2]),
        )

    class w_copy:
        def __init__(self, i, quarter=None):
            r0, nr, s0 = (0, 8, 0) if quarter is None else (4 * quarter, 4, 2 * quarter)
            self.cps = [pltpu.make_async_copy(
                w_u32[i // 2].at[:, par, pl.ds((i % 2) * 8 + r0, nr), :],
                stage4.at[2 * (i % NSLOT) + par, :, pl.ds(r0, nr), :],
                sem_w.at[i % NSLOT, s0 + par]) for par in range(2)]

        def start(self):
            for cp in self.cps:
                cp.start()

        def wait(self):
            for cp in self.cps:
                cp.wait()

    def wo_copy(n):
        return pltpu.make_async_copy(wo_u32.at[:, pl.ds(n * 128, 128)], wo_v.at[n], sem_o.at[n])

    def x_copy(half):
        rows = pl.ds(half * (S // 2), S // 2)
        return pltpu.make_async_copy(x_hbm.at[rows, :], x_v.at[rows, :], sem_x.at[1 + half])

    def out_copy(r0, nr, k):
        return pltpu.make_async_copy(out_v.at[pl.ds(r0, nr), :], out_hbm.at[pl.ds(r0, nr), :], sem_out.at[k])

    x0_copy = pltpu.make_async_copy(x_hbm.bitcast(U32).at[pl.ds(0, PM // 2), :], x0, sem_x.at[0])
    x0_copy.start()
    w_copy(0, 0).start()

    r = lax.broadcasted_iota(jnp.int32, (256, 128), 0)
    t = lax.broadcasted_iota(jnp.int32, (256, 128), 1)
    rr = r & 127
    f = jnp.where(rr < 64, 2 * rr, 2 * (rr - 64) + 1)
    n = ((2 * f + 1) * t + jnp.where(r >= 128, 128, 0)) & 511
    fmat[...] = jnp.cos(n.astype(F32) * (2.0 * math.pi / 512.0)).astype(BF16)
    r = lax.broadcasted_iota(jnp.int32, (128, 256), 1)
    t = lax.broadcasted_iota(jnp.int32, (128, 256), 0)
    rr = r & 127
    f = jnp.where(rr < 64, 2 * rr, 2 * (rr - 64) + 1)
    n = ((2 * f + 1) * t + jnp.where(r >= 128, 128, 0)) & 511
    gmat[...] = (jnp.cos(n.astype(F32) * (2.0 * math.pi / 512.0)) * (1.0 / 128.0)).astype(BF16)

    def head_and_pos(idx):
        second = jnp.logical_or(jnp.logical_and(idx >= MEM, idx < 2 * MEM), idx >= 2 * MEM + SEG)
        pos = jnp.where(idx < 2 * MEM, jnp.where(second, idx - MEM, idx),
                        jnp.where(second, idx - MEM - SEG, idx - MEM))
        return second, pos

    qh, ql = head_and_pos(lax.broadcasted_iota(jnp.int32, (PR, PR), 0))
    kh, kl = head_and_pos(lax.broadcasted_iota(jnp.int32, (PR, PR), 1))
    ok = jnp.logical_and(qh == kh, jnp.logical_or(ql < MEM, ql >= kl))
    bias[...] = jnp.where(ok, 0.0, jnp.where(qh == kh, -1e9, -jnp.inf)).astype(F32)

    zsm[0] = 0
    prm[0:1, :] = dvec_ref[...].astype(F32).reshape(1, D)
    prm[1:2, :] = gw_ref[...].astype(F32).reshape(1, D)
    kpad[0:8, :] = jnp.zeros((8, 128), F32)
    obuf[0:TPS, :] = jnp.zeros((TPS, H * DH), BF16)

    def relayout(q, k, zero, always, m, dbl):
        base = ((q // 8) % NSLOT) * (D * 8) + q % 8
        low = jnp.full((RG, DH), 0xFFFF, U32)
        high = jnp.full((RG, DH), 0xFFFF0000, U32)
        m = low if m is None else jnp.where(always, low, m)
        for r0 in range(0, D // 2, RG):
            a = stage[pl.ds(base + r0 * 8, RG, stride=8), :]
            b = stage[pl.ds(base + D * 4 + r0 * 8, RG, stride=8), :]
            lo = (a & m) | (b << 16)
            if always is not None:
                hi = (a >> 16) | (b & (jnp.where(always, high, lo) if dbl else high))
                m = jnp.where(always, low, hi if dbl else (lo ^ hi if RMODE == 'xor' else lo))
            else:
                hi = (a >> 16) | (b & high)
            wtmp[k][zero, r0:r0 + RG, :] = lo
            wtmp[k][zero + 1, r0:r0 + RG, :] = hi
            wqkv[2 * q, r0:r0 + RG, :] = lo
            wqkv[2 * q + 1, r0:r0 + RG, :] = hi
        return m

    def proj(q0, su, zero):
        j = 2 * q0 + su // 4
        for r0, nr in MSUB[su % 4]:
            wj = pltpu.bitcast(wtmp[su // 8][(su // 4) % 2], BF16)
            res = jnp.dot(pltpu.bitcast(x0[r0 // 2:(r0 + nr) // 2, :], BF16), wj,
                          preferred_element_type=F32)
            ring[j, r0:r0 + nr, :] = res.astype(BF16)

    x0_copy.wait()
    w_copy(0, 0).wait()
    w_copy(0, 1).start()
    w_copy(1).start()

    def pro_a(c, carry):
        @pl.when(c == 1)
        def _():
            w_copy(0, 1).wait()
            for cp in conv_copies(0, 0):
                cp.start()
        zero = zsm[0]
        always = jnp.full((8, 128), zero, jnp.int32) == 0
        q0 = c * PPA
        relayout(q0, 0, zero, None, None, False)
        for su in range(8 * PPA):
            proj(q0, su, zero)
            if su % 8 == 0 and su // 8 + 1 < PPA:
                relayout(q0 + su // 8 + 1, su // 8 + 1, zero, always, None, True)
        return carry

    if "pre" in phases:
        lax.fori_loop(0, 8 // PPA, pro_a, 0)
    else:
        w_copy(0, 1).wait()
        for cp in conv_copies(0, 0):
            cp.start()

    W_WAIT = {1: 0, 2: 1, 3: 3, 4: 4, 5: 6}
    W_START = {2: 0, 3: 1, 4: 2, 5: 4}
    for i in range(1, NCHUNK):
        assert W_WAIT[i] == min(c for c in range(NCH) if (8 + PPI * c + PPI - 1) // 8 >= i)
    for i, c0 in W_START.items():
        assert c0 < W_WAIT[i]
        assert all((8 + PPI * c) // 8 > i - NSLOT for c in range(c0, NCH))

    def pro_b(c, carry):
        slot = c % 2
        for i, cw in W_WAIT.items():
            @pl.when(c == cw)
            def _(i=i):
                w_copy(i).wait()
        for cp in conv_copies(c, slot):
            cp.wait()

        @pl.when(c + 1 < NCH)
        def _():
            for cp in conv_copies(c + 1, 1 - slot):
                cp.start()
        for i, cs in W_START.items():
            @pl.when(c == cs)
            def _(i=i):
                w_copy(i).start()
        for cs, n0 in ((3, 0), (5, 4)):
            @pl.when(c == cs)
            def _(n0=n0):
                for n in range(n0, n0 + 4):
                    wo_copy(n).start()

        @pl.when(c == 6)
        def _():
            for half in range(2):
                x_copy(half).start()

        zero = zsm[0]
        always = jnp.full((8, 128), zero, jnp.int32) == 0
        zrow = pl.multiple_of(zero * 16, 16)
        col = pl.multiple_of(c * 128, 128)
        w = shift_ref[:, pl.ds(col, 128)].astype(F32)
        dv = prm[0:1, pl.ds(col, 128)]
        q0 = 8 + c * PPI

        w3 = jnp.broadcast_to(w[3:4], (KG, 128))
        pace = [w3]
        gate = [None]

        def kv_mul(j):
            if gate[0] is not None:
                pace[0] = jnp.where(always, w3, pltpu.bitcast(gate[0], F32))
            for r0 in range(j * CB, (j + 1) * CB, 2 * KG):
                kpad[8 + r0:8 + r0 + 2 * KG, :] = kin[slot, r0:r0 + 2 * KG, :].astype(F32)
                vf = vin[slot, r0:r0 + 2 * KG, :].astype(F32)
                kvs = []
                for hf in range(2):
                    base = 8 + r0 + hf * KG
                    ks = (kpad[base - 3:base - 3 + KG, :] * pace[0] + kpad[base - 2:base - 2 + KG, :] * w[2:3]
                          + kpad[base - 1:base - 1 + KG, :] * w[1:2] + kpad[base:base + KG, :] * w[0:1])
                    kv = ks * vf[hf * KG:(hf + 1) * KG]
                    if hf == 1 or KVLINK == 1:
                        pace[0] = jnp.where(always, w3, kv)
                    kvs.append(kv)
                rr0 = r0 % (4 * CB)
                kvb[j // 4][pl.ds(zrow + rr0, 2 * KG), :] = jnp.concatenate(kvs, axis=0).astype(BF16)
            gate[0] = pltpu.bitcast(pace[0], U32)

        def kv_load(j):
            return kvb[j // 4][(j % 4) * CB:(j % 4 + 1) * CB, :]

        def u_dft(j):
            spec[zero + j] = jnp.dot(fmat[...], kv_load(j), preferred_element_type=F32)

        def h_dft():
            for m in range(NB):
                spec[zero + NB + m] = lax.dot_general(fmat[...], hin[slot, :, m * CB:(m + 1) * CB],
                                               (((1,), (1,)), ((), ())), preferred_element_type=F32)

        def ld(idx, r0):
            return spec[idx, r0:r0 + GR, :]

        def freq_mul(i):
            for g in range(0, 128, GR):
                sgn = 1.0 if g < 64 else -1.0
                hr1, hi1 = ld(NB + i + 1, g), ld(NB + i + 1, 128 + g)
                if gate[0] is not None and GATEZ:
                    gt = pltpu.bitcast(gate[0], F32)
                    hr1 = jnp.concatenate([jnp.where(always, hr1[0:8], gt), hr1[8:]], axis=0) if GR > 8 else jnp.where(always, hr1, gt)
                    gate[0] = None
                y0r = y0i = y1r = y1i = None
                for j in range(i + 2):
                    ur, ui = ld(j, g), ld(j, 128 + g)
                    tr = ur * hr1 - ui * hi1
                    ti = ur * hi1 + ui * hr1
                    y1r, y1i = (tr, ti) if y1r is None else (y1r + tr, y1i + ti)
                    if j <= i:
                        hr1, hi1 = ld(NB + i - j, g), ld(NB + i - j, 128 + g)
                        tr = ur * hr1 - ui * hi1
                        ti = ur * hi1 + ui * hr1
                        y0r, y0i = (tr, ti) if y0r is None else (y0r + tr, y0i + ti)
                if sgn > 0:
                    z1r, z1i = y1r - y0i, y1i + y0r
                else:
                    z1r, z1i = y1r + y0i, y1i - y0r
                if i > 0:
                    pr_, pi_ = ld(2 * NB, g), ld(2 * NB, 128 + g)
                    if sgn > 0:
                        y0r, y0i = y0r - pi_, y0i + pr_
                    else:
                        y0r, y0i = y0r + pi_, y0i - pr_
                if i + 2 < NB:
                    spec[zero + 2 * NB, g:g + GR, :] = y1r
                    spec[zero + 2 * NB, 128 + g:128 + g + GR, :] = y1i
                zi = zero + 2 * NB + 1 + i // 2
                h2 = GR // 2
                spec[zi, g // 2:g // 2 + h2, :] = pltpu.bitcast(y0r.astype(BF16), F32)
                spec[zi, 64 + g // 2:64 + g // 2 + h2, :] = pltpu.bitcast(y0i.astype(BF16), F32)
                spec[zi, 128 + g // 2:128 + g // 2 + h2, :] = pltpu.bitcast(z1r.astype(BF16), F32)
                spec[zi, 192 + g // 2:192 + g // 2 + h2, :] = pltpu.bitcast(z1i.astype(BF16), F32)

        def inv(i):
            r0 = (i % 2) * 128
            z = pltpu.bitcast(spec[2 * NB + 1 + i // 2, r0:r0 + 128, :], BF16)
            y = jnp.dot(gmat[...], z, preferred_element_type=F32)
            y = y + kv_load(i).astype(F32) * dv
            ybuf[i * CB:(i + 1) * CB, pl.ds(col, 128)] = y.astype(BF16)

        do_c = "conv" in phases
        do_p = "pre" in phases
        def side(tok):
            if tok[0] == "k" and do_c:
                for j in range(4 * tok[1], 4 * tok[1] + 4):
                    kv_mul(j)
            if tok[0] == "r" and do_p:
                gate[0] = relayout(q0 + tok[1], tok[1], zero, always, gate[0], RMODE == 'dbl')

        if do_p:
            relayout(q0, 0, zero, None, None, False)
        if do_c:
            h_dft()
        for tok in SIDE:
            side(tok)
        for su in range(8 * PPI):
            if do_p:
                proj(q0, su, zero)
            if do_c:
                if su in U_AFTER:
                    for j in range(U_AFTER.index(su) * 4, U_AFTER.index(su) * 4 + 4):
                        u_dft(j)
                for i in INV_AFTER.get(su + 1, ())[:1]:
                    freq_mul(i)
                for i in INV_AFTER.get(su, ()):
                    inv(i)
        return carry

    lax.fori_loop(0, NCH, pro_b, 0)
    for half in range(2):
        x_copy(half).wait()
    for n in range(8):
        wo_copy(n).wait()

    lhs_q[0:MEM, :] = mem0_ref[...]
    gw = prm[1:2, :]
    scale = DH ** -0.5
    always = jnp.full((8, 128), zsm[0], jnp.int32) == 0

    def combine(b, rows_start, nrows):
        xt = x_v[pl.ds(rows_start, nrows), :].astype(F32)
        g = jax.nn.sigmoid(jnp.sum(xt * gw, axis=-1, keepdims=True))
        a = xt * ybuf[pl.ds(rows_start, nrows), :].astype(F32)
        res = g * a + (1.0 - g) * b
        out_v[pl.ds(rows_start, nrows), :] = res.astype(BF16)
        return res

    def step(s, defer, early, gate):
        p = pl.multiple_of(jnp.minimum(P0 + TPS * s, S - TPS), 8)
        lag = pl.multiple_of(jnp.maximum(TPS * (s - 1), 0), 8)
        lhs_q[MEM:, :] = x_v[pl.ds(p, TPS), :]
        lhs = [lhs_q[:, 0:D // 2], lhs_q[:, D // 2:]]
        cur = pl.multiple_of((s % RING) * SEG, SEG)
        offs = [pl.multiple_of((p + 8 * k) % (RING * SEG), 8) for k in range(TPS // 8)]
        tok0 = pl.multiple_of(s * SEG, SEG)

        def fetch(pr):
            lhs_o[MEM:, pr * 256:(pr + 1) * 256] = obuf[pl.ds(lag, TPS), pr * 256:(pr + 1) * 256]
            for tsel in range(3):
                for hh in range(2):
                    t0 = 2 * MEM + hh * SEG
                    cbuf[tsel * 16 + pr, t0:t0 + SEG, :] = ring[tsel * H + 2 * pr + hh, pl.ds(cur, SEG), :]

        part = {}

        def qkv(pr, tsel, hh, half=None):
            j = tsel * H + 2 * pr + hh
            for hf in ((0, 1) if half is None else (half,)):
                wj = wqkv[j, hf * (D // 4):(hf + 1) * (D // 4), :]
                if gate is not None and (pr, tsel, hh, hf) == (GATEPR, 0, 0, 0):
                    wj = jnp.concatenate([jnp.where(always, wj[0:8], gate), wj[8:]], axis=0)
                wj = pltpu.bitcast(wj, BF16)
                t = jnp.dot(lhs[hf], wj, preferred_element_type=F32)
                part[j] = t if hf == 0 else t + part[j]
            if half == 0:
                return
            res = part.pop(j).astype(BF16)
            cbuf[tsel * 16 + pr, hh * MEM:(hh + 1) * MEM, :] = res[0:MEM]
            for k in range(TPS // 8):
                ring[j, pl.ds(offs[k], 8), :] = res[MEM + 8 * k:MEM + 8 * (k + 1)]

        probs = {}

        def scores(pr):
            qp = cbuf[pr]
            kp = cbuf[16 + pr]
            sc = lax.dot_general(qp, kp, (((1,), (1,)), ((), ())), preferred_element_type=F32) * scale
            fill = bias[...]
            sc = jnp.where(fill == 0.0, sc, fill)
            mx = jnp.max(sc, axis=-1, keepdims=True)
            e = jnp.exp(sc - mx)
            den = jnp.sum(e, axis=-1, keepdims=True)
            rc = pl.reciprocal(den, approx=True)
            rc = rc * (2.0 - den * rc)
            probs[pr] = (e * rc).astype(BF16)

        def pv(pr, mem_rows=True, tok_rows=True):
            r0 = 0 if mem_rows else 2 * MEM
            r1 = PR if tok_rows else 2 * MEM
            o = jnp.dot(probs[pr][r0:r1], cbuf[32 + pr], preferred_element_type=F32).astype(BF16)
            for hh in range(2):
                c0 = (2 * pr + hh) * DH
                if mem_rows:
                    lhs_o[0:MEM, c0:c0 + DH] = o[hh * MEM:(hh + 1) * MEM]
                if tok_rows:
                    t0 = 2 * MEM + hh * SEG - r0
                    obuf[pl.ds(tok0, SEG), c0:c0 + DH] = o[t0:t0 + SEG]

        accs = [None] * (D // 128)

        def wo(pr, half):
            lo = lhs_o[:, pr * 256:(pr + 1) * 256]
            for nb in range(half * 4, half * 4 + 4):
                wt = pltpu.bitcast(wo_v[nb, pr * 128:(pr + 1) * 128, :], BF16)
                t = jnp.dot(lo, wt, preferred_element_type=F32)
                accs[nb] = t if accs[nb] is None else t + accs[nb]

        NP = H // 2
        late = ()
        main = [("q", pr, t, h) for pr in range(NP) for t in range(3) for h in range(2)]
        if early:
            fetch(0)
            for t in range(3):
                for h in range(2):
                    qkv(0, t, h, 0)
        nt = NP - NDEFER if defer else NP
        main += [("w", pr, hf) for pr in range(nt) for hf in range(2)]
        main += [("w", pr, hf) for hf in range(2) for pr in range(nt, NP)]
        ns = npv = 0
        s_at, pv_at = {}, {}
        for slot, item in enumerate(main):
            if item[0] == "w":
                while item[1] not in pv_at:
                    if npv == ns:
                        scores(ns)
                        s_at[ns] = slot
                        ns += 1
                    pv(npv, tok_rows=npv not in late)
                    pv_at[npv] = slot
                    npv += 1
                wo(item[1], item[2])
            else:
                if early and item[1] == 0:
                    qkv(*item[1:], 1)
                else:
                    if item[2] == 0 and item[3] == 0:
                        fetch(item[1])
                    qkv(*item[1:])
            if GROUP == 1:
                if ns < NP and slot + 1 >= 6 * ns + DS:
                    scores(ns)
                    s_at[ns] = slot + 1
                    ns += 1
                if npv < ns and slot + 1 >= s_at[npv] + DPV:
                    pv(npv, tok_rows=npv not in late)
                    pv_at[npv] = slot + 1
                    npv += 1
            elif (slot + 1 - DS) % (6 * GROUP) == 0:
                order = []
                for _ in range(GROUP):
                    if npv < ns and slot + 1 >= s_at[npv] + DPV:
                        order.append(("p", npv))
                        pv_at[npv] = slot + 1
                        npv += 1
                for _ in range(GROUP):
                    if ns < NP and slot + 1 >= 6 * ns + DS:
                        order.append(("s", ns))
                        s_at[ns] = slot + 1
                        ns += 1
                if SFIRST:
                    order = order[::-1]
                for kind, idx in order:
                    if kind == "s":
                        scores(idx)
                    else:
                        pv(idx)
        for pr in late:
            pv(pr, mem_rows=False)
        for nb in range(D // 128):
            lhs_q[0:MEM, nb * 128:(nb + 1) * 128] = accs[nb][0:MEM].astype(BF16)
        acc = jnp.concatenate(accs, axis=1)
        res = combine(acc[MEM:], lag, TPS)
        tk = None
        for r in range(0, TPS, 8):
            for cc in range(0, D, 128):
                t = pltpu.bitcast(res[r:r + 8, cc:cc + 128], U32)
                tk = t if tk is None else tk ^ t
        return tk

    def steps(it, carry):
        s0 = it * UNROLL

        @pl.when(jnp.logical_and(s0 % 8 == OTRIG, s0 > 8))
        def _():
            k = s0 // 8 - 1
            out_copy(pl.multiple_of(k * OCH, OCH), OCH, k).start()

        gate = None
        for u in range(UNROLL):
            gate = step(s0 + u, u + 1 < UNROLL, u > 0, gate if GATEPR >= 0 else None)
        return carry

    nstream = (NSEG - 1) // 8
    if "main" in phases:
        lax.fori_loop(0, NSEG // UNROLL, steps, 0)
    else:
        if "main1" in phases:
            lax.fori_loop(0, 1 + zsm[0], steps, 0)
        for k in range(nstream):
            out_copy(k * OCH, OCH, k).start()
    tail0 = nstream * OCH
    out_copy(tail0, EPI[0][0] - tail0, nstream).start()

    for e, (a0, na) in enumerate(EPI):
        if "epi" in phases:
            lo = obuf[a0:a0 + na, :]
            b = jnp.concatenate(
                [jnp.dot(lo, pltpu.bitcast(wo_v[nb], BF16), preferred_element_type=F32)
                 for nb in range(D // 128)], axis=1)
            combine(b, a0, na)
        out_copy(a0, na, nstream + 1 + e).start()
    for k in range(nstream):
        out_copy(k * OCH, OCH, k).wait()
    out_copy(tail0, EPI[0][0] - tail0, nstream).wait()
    for e, (a0, na) in enumerate(EPI):
        out_copy(a0, na, nstream + 1 + e).wait()


def build(phases=("conv", "pre", "main", "epi")):
    @functools.partial(jax.jit, static_argnames=("B_seg_len",))
    def fn(A_q, A_k, A_v, A_shift_k, A_ssm_k, A_ssm_D, B_x, B_mem0, B_Wq, B_Wk, B_Wv, B_Wo,
           B_seg_len, gate_w):
        assert int(B_seg_len) == SEG
        any_spec = pl.BlockSpec(memory_space=pl.ANY)
        vm = pl.BlockSpec(memory_space=pltpu.VMEM)
        out = pl.pallas_call(
            functools.partial(_kernel, phases),
            out_shape=jax.ShapeDtypeStruct((S, D), BF16),
            in_specs=[any_spec] * 8 + [vm] * 4,
            out_specs=any_spec,
            scratch_shapes=[
                pltpu.VMEM((S, D), BF16),
                pltpu.VMEM((PM // 2, D), U32),
                pltpu.VMEM((S, D), BF16),
                pltpu.VMEM((S, D), BF16),
                pltpu.VMEM((3 * H, D // 2, DH), U32),
                pltpu.VMEM((2, D // 2, DH), U32),
                pltpu.VMEM((2, D // 2, DH), U32),
                pltpu.VMEM((2, D // 2, DH), U32),
                pltpu.VMEM((2, D // 2, DH), U32),
                pltpu.VMEM((2, D // 2, DH), U32),
                pltpu.VMEM((S // 4, 128), BF16),
                pltpu.VMEM((S // 4, 128), BF16),
                pltpu.VMEM((S // 4, 128), BF16),
                pltpu.VMEM((S // 4, 128), BF16),
                pltpu.VMEM((D // 128, H * DH // 2, 128), U32),
                pltpu.VMEM((NSLOT * D * 8, DH), U32),
                pltpu.VMEM((3 * H, RING * SEG, DH), BF16),
                pltpu.VMEM((3 * 16, PR, DH), BF16),
                pltpu.VMEM((S, H * DH), BF16),
                pltpu.VMEM((MEM + TPS, D), BF16),
                pltpu.VMEM((MEM + TPS, H * DH), BF16),
                pltpu.VMEM((2, S, 128), BF16),
                pltpu.VMEM((2, S, 128), BF16),
                pltpu.VMEM((2, 128, S), BF16),
                pltpu.VMEM((S + 8, 128), F32),
                pltpu.VMEM((2 * NB + 1 + NB // 2, 256, 128), F32),
                pltpu.VMEM((256, 128), BF16),
                pltpu.VMEM((128, 256), BF16),
                pltpu.VMEM((PR, PR), F32),
                pltpu.VMEM((8, D), F32),
                pltpu.SMEM((1,), jnp.int32),
                pltpu.SemaphoreType.DMA((2, 3)),
                pltpu.SemaphoreType.DMA((3,)),
                pltpu.SemaphoreType.DMA((NSLOT, 4)),
                pltpu.SemaphoreType.DMA((8,)),
                pltpu.SemaphoreType.DMA((12,)),
            ],
            compiler_params=pltpu.CompilerParams(vmem_limit_bytes=120 * 1024 * 1024),
        )(A_q.reshape(S, D), A_k.reshape(S, D), A_v.reshape(S, D), A_ssm_k,
          B_Wq.reshape(D // 2, 2, H, DH), B_Wk.reshape(D // 2, 2, H, DH), B_Wv.reshape(D // 2, 2, H, DH),
          B_Wo.reshape(H * DH, D),
          A_shift_k.T, A_ssm_D, gate_w, B_mem0.reshape(MEM, D))
        return out.reshape(1, S, D)
    return fn


pallas_gated_mix__ssm_conv_h3__memory_aug_recurrent_mem_tr__prompt_kernel = build()
```

```python
import functools
import math

import jax
import jax.numpy as jnp
from jax import lax
import jax.experimental.pallas as pl
import jax.experimental.pallas.tpu as pltpu

F32 = jnp.float32
BF16 = jnp.bfloat16
U32 = jnp.uint32

S = 2048
D = 1024
H = 32
DH = 128
MEM = 8
SEG = 32
NSEG = S // SEG
TPS = 24
PM = S - TPS * (NSEG - 1) - MEM
RING = 18
PR = 2 * (MEM + SEG)
CB = 128
NB = S // CB
NCH = D // 128
DS = 7
DPV = 9
RMODE = 'none'
KVLINK = 1
GATEZ = False
UNROLL = 2
NDEFER = 5
GATEPR = 2
GROUP = 1
SFIRST = False
OTRIG = UNROLL % 8
PPA = 8
USE_WTMP = False
DMAPOS = -1
PPI = 5
RG = 8
SIDE = (('k', 0), ('k', 1), ('k', 2), ('k', 3), ('r', 1), ('r', 2), ('r', 3), ('r', 4))
U_AFTER = (2, 3, 5, 6)
KG = 8
GR = 16
MSUB = (((0, 144),), ((144, 128),), ((272, 128),), ((400, 128),))
INV_AFTER = {12: (0, 1), 14: (2, 3), 16: (4, 5), 19: (6, 7), 23: (8, 9), 28: (10, 11), 33: (12, 13), 39: (14, 15)}


def _pair_of(c, k):
    return ((0, PPA + c), (1, 2 * c), (1, 2 * c + 1), (2, 2 * c), (2, 2 * c + 1))[k]


_SLOT = {(0, hp): hp for hp in range(PPA)}
_SLOT.update({_pair_of(c, k): PPA + PPI * c + k for c in range(NCH) for k in range(PPI)})

XA = 144
A_WAIT = {0: (1,), 1: (2,), 2: (3,), 3: (4, 5), 5: (6, 7)}
A_START = {0: (("a", 3),), 1: (("a", 4), ("a", 5)), 2: (("a", 6), ("a", 7)), 3: (("c", 0), ("c", 1), ("c", 2)),
           5: (("b", 0), ("b", 1), ("b", 2), ("b", 3), ("b", 4))}
OCH = 192
EPI = ((1488, 144), (1632, 144), (1776, 144), (1920, 128))


def _kernel(phases,
            x_hbm, k_hbm, v_hbm, h_hbm, wq_hbm, wk_hbm, wv_hbm, wo_hbm,
            shift_ref, dvec_ref, gw_ref, mem0_ref,
            out_hbm,
            x_v, x0, ybuf, out_v, wqkv, wt0, wt1, wt2, wt3, wt4, kv0, kv1, kv2, kv3, wo_v, ring, cbuf, obuf, lhs_q, lhs_o,
            kin, vin, hin, kpad, spec, fmat, gmat, bias, prm, zsm,
            sem_c, sem_x, sem_w, sem_o, sem_out):
    w_u32 = tuple(w.bitcast(U32) for w in (wq_hbm, wk_hbm, wv_hbm))
    wo_u32 = wo_hbm.bitcast(U32)
    wtmp = (wt0, wt1, wt2, wt3, wt4)
    kvb = (kv0, kv1, kv2, kv3)

    def conv_copy(c, slot, n):
        if n == 2:
            return pltpu.make_async_copy(h_hbm.at[pl.ds(c * 128, 128), :], hin.at[slot], sem_c.at[slot, 2])
        src, dst = ((k_hbm, kin), (v_hbm, vin))[n]
        return pltpu.make_async_copy(src.at[:, pl.ds(c * 128, 128)], dst.at[slot], sem_c.at[slot, n])

    def conv_copies(c, slot):
        return [conv_copy(c, slot, n) for n in range(3)]

    class w_copy:
        def __init__(self, mat, hp, slot, sem):
            self.cps = [pltpu.make_async_copy(
                w_u32[mat].at[:, par, hp, :], wqkv.at[2 * slot + par], sem_w.at[sem, par])
                for par in range(2)]

        def start(self):
            for cp in self.cps:
                cp.start()

        def wait(self):
            for cp in self.cps:
                cp.wait()

    def wa_copy(hp):
        return w_copy(0, hp, hp, hp)

    def wb_copy(c, k):
        mat, hp = _pair_of(c, k)
        hp = min(hp, H // 2 - 1) if isinstance(hp, int) else jnp.minimum(hp, H // 2 - 1)
        return w_copy(mat, hp, PPA + PPI * c + k, PPA + (c % 2) * PPI + k)

    def wo_copy(n):
        return pltpu.make_async_copy(wo_u32.at[:, pl.ds(n * 128, 128)], wo_v.at[n], sem_o.at[n])

    def x_copy(n):
        r0 = n * (S // NCH)
        rows = pl.ds(r0 if isinstance(n, int) else pl.multiple_of(r0, S // NCH), S // NCH)
        return pltpu.make_async_copy(x_hbm.at[rows, :], x_v.at[rows, :], sem_x.at[2 + n])

    def out_copy(r0, nr, k):
        return pltpu.make_async_copy(out_v.at[pl.ds(r0, nr), :], out_hbm.at[pl.ds(r0, nr), :], sem_out.at[k])

    def x0_copy(part):
        rows = pl.ds(0, XA // 2) if part == 0 else pl.ds(XA // 2, (PM - XA) // 2)
        return pltpu.make_async_copy(x_hbm.bitcast(U32).at[rows, :], x0.at[rows, :], sem_x.at[part])

    x0_copy(0).start()
    wa_copy(0).start()

    r = lax.broadcasted_iota(jnp.int32, (256, 128), 0)
    t = lax.broadcasted_iota(jnp.int32, (256, 128), 1)
    rr = r & 127
    f = jnp.where(rr < 64, 2 * rr, 2 * (rr - 64) + 1)
    n = ((2 * f + 1) * t + jnp.where(r >= 128, 128, 0)) & 511
    fmat[...] = jnp.cos(n.astype(F32) * (2.0 * math.pi / 512.0)).astype(BF16)
    x0_copy(1).start()
    wa_copy(1).start()
    r = lax.broadcasted_iota(jnp.int32, (128, 256), 1)
    t = lax.broadcasted_iota(jnp.int32, (128, 256), 0)
    rr = r & 127
    f = jnp.where(rr < 64, 2 * rr, 2 * (rr - 64) + 1)
    n = ((2 * f + 1) * t + jnp.where(r >= 128, 128, 0)) & 511
    gmat[...] = (jnp.cos(n.astype(F32) * (2.0 * math.pi / 512.0)) * (1.0 / 128.0)).astype(BF16)

    def head_and_pos(idx):
        second = jnp.logical_or(jnp.logical_and(idx >= MEM, idx < 2 * MEM), idx >= 2 * MEM + SEG)
        pos = jnp.where(idx < 2 * MEM, jnp.where(second, idx - MEM, idx),
                        jnp.where(second, idx - MEM - SEG, idx - MEM))
        return second, pos

    qh, ql = head_and_pos(lax.broadcasted_iota(jnp.int32, (PR, PR), 0))
    kh, kl = head_and_pos(lax.broadcasted_iota(jnp.int32, (PR, PR), 1))
    ok = jnp.logical_and(qh == kh, jnp.logical_or(ql < MEM, ql >= kl))
    bias[...] = jnp.where(ok, 0.0, jnp.where(qh == kh, -1e9, -jnp.inf)).astype(F32)

    zsm[0] = 0
    prm[0:1, :] = dvec_ref[...].astype(F32).reshape(1, D)
    prm[1:2, :] = gw_ref[...].astype(F32).reshape(1, D)
    kpad[0:8, :] = jnp.zeros((8, 128), F32)
    obuf[0:TPS, :] = jnp.zeros((TPS, H * DH), BF16)

    def relayout(sl, k, zero, always, m, dbl):
        low = jnp.full((RG, DH), 0xFFFF, U32)
        high = jnp.full((RG, DH), 0xFFFF0000, U32)
        m = low if m is None else jnp.where(always, low, m)
        for r0 in range(0, D // 2, RG):
            a = wqkv[2 * sl, r0:r0 + RG, :]
            b = wqkv[2 * sl + 1, r0:r0 + RG, :]
            lo = (a & m) | (b << 16)
            if always is not None and (RMODE != 'none' or dbl):
                hi = (a >> 16) | (b & (jnp.where(always, high, lo) if dbl else high))
                m = jnp.where(always, low, hi if dbl else (lo ^ hi if RMODE == 'xor' else lo))
            else:
                hi = (a >> 16) | (b & high)
            if USE_WTMP:
                wtmp[k][zero, r0:r0 + RG, :] = lo
                wtmp[k][zero + 1, r0:r0 + RG, :] = hi
            wqkv[2 * sl, r0:r0 + RG, :] = lo
            wqkv[2 * sl + 1, r0:r0 + RG, :] = hi
        return m

    def proj(mat, hp, sl, k, hh, ms):
        for r0, nr in MSUB[ms]:
            wj = pltpu.bitcast(wtmp[k][hh] if USE_WTMP else wqkv[2 * sl + hh], BF16)
            res = jnp.dot(pltpu.bitcast(x0[r0 // 2:(r0 + nr) // 2, :], BF16), wj,
                          preferred_element_type=F32)
            ring[mat * H + 2 * hp + hh, r0:r0 + nr, :] = res.astype(BF16)

    zero = zsm[0]
    always = jnp.full((8, 128), zero, jnp.int32) == 0
    do_p = "pre" in phases
    x0_copy(0).wait()
    wa_copy(0).wait()
    wa_copy(2).start()
    if do_p:
        relayout(0, 0, zero, None, None, False)
        proj(0, 0, 0, 0, 0, 0)
        proj(0, 0, 0, 0, 1, 0)
    x0_copy(1).wait()
    for hp in range(PPA):
        for n in A_WAIT.get(hp, ()):
            wa_copy(n).wait()
        for st in A_START.get(hp, ()):
            if st[0] == "a":
                wa_copy(st[1]).start()
            elif st[0] == "b":
                wb_copy(0, st[1]).start()
            else:
                conv_copy(0, 0, st[1]).start()
        for su in range(8):
            hh, ms = (su % 2, su // 2) if hp == 0 else (su // 4, su % 4)
            if do_p and not (hp == 0 and ms == 0):
                proj(0, hp, hp, hp % PPI, hh, ms)
            if do_p and su == (2 if hp == 0 else 0) and hp + 1 < PPA:
                relayout(hp + 1, (hp + 1) % PPI, zero, always, None, True)

    def pro_b(c, carry):
        slot = c % 2
        for k in range(PPI):
            wb_copy(c, k).wait()
        for cp in conv_copies(c, slot):
            cp.wait()

        def prefetch():
            for cp in conv_copies(jnp.minimum(c + 1, NCH - 1), 1 - slot):
                cp.start()
            for k in range(PPI):
                wb_copy(c + 1, k).start()
            wo_copy(c).start()
            x_copy(c).start()

        if DMAPOS < 0:
            prefetch()
        zero = zsm[0]
        always = jnp.full((8, 128), zero, jnp.int32) == 0
        zrow = pl.multiple_of(zero * 16, 16)
        col = pl.multiple_of(c * 128, 128)
        w = shift_ref[:, pl.ds(col, 128)].astype(F32)
        dv = prm[0:1, pl.ds(col, 128)]
        sl0 = PPA + c * PPI

        w3 = jnp.broadcast_to(w[3:4], (KG, 128))
        pace = [w3]
        gate = [None]

        def kv_mul(j):
            if gate[0] is not None:
                pace[0] = jnp.where(always, w3, pltpu.bitcast(gate[0], F32))
            for r0 in range(j * CB, (j + 1) * CB, 2 * KG):
                kpad[8 + r0:8 + r0 + 2 * KG, :] = kin[slot, r0:r0 + 2 * KG, :].astype(F32)
                vf = vin[slot, r0:r0 + 2 * KG, :].astype(F32)
                kvs = []
                for hf in range(2):
                    base = 8 + r0 + hf * KG
                    ks = (kpad[base - 3:base - 3 + KG, :] * pace[0] + kpad[base - 2:base - 2 + KG, :] * w[2:3]
                          + kpad[base - 1:base - 1 + KG, :] * w[1:2] + kpad[base:base + KG, :] * w[0:1])
                    kv = ks * vf[hf * KG:(hf + 1) * KG]
                    if hf == 1 or KVLINK == 1:
                        pace[0] = jnp.where(always, w3, kv)
                    kvs.append(kv)
                rr0 = r0 % (4 * CB)
                kvb[j // 4][pl.ds(zrow + rr0, 2 * KG), :] = jnp.concatenate(kvs, axis=0).astype(BF16)
            gate[0] = pltpu.bitcast(pace[0], U32)

        def kv_load(j):
            return kvb[j // 4][(j % 4) * CB:(j % 4 + 1) * CB, :]

        def u_dft(j):
            spec[zero + j] = jnp.dot(fmat[...], kv_load(j), preferred_element_type=F32)

        def h_dft():
            for m in range(NB):
                spec[zero + NB + m] = lax.dot_general(fmat[...], hin[slot, :, m * CB:(m + 1) * CB],
                                               (((1,), (1,)), ((), ())), preferred_element_type=F32)

        def ld(idx, r0):
            return spec[idx, r0:r0 + GR, :]

        def freq_mul(i):
            for g in range(0, 128, GR):
                sgn = 1.0 if g < 64 else -1.0
                hr1, hi1 = ld(NB + i + 1, g), ld(NB + i + 1, 128 + g)
                if gate[0] is not None and GATEZ:
                    gt = pltpu.bitcast(gate[0], F32)
                    hr1 = jnp.concatenate([jnp.where(always, hr1[0:8], gt), hr1[8:]], axis=0) if GR > 8 else jnp.where(always, hr1, gt)
                    gate[0] = None
                y0r = y0i = y1r = y1i = None
                for j in range(i + 2):
                    ur, ui = ld(j, g), ld(j, 128 + g)
                    tr = ur * hr1 - ui * hi1
                    ti = ur * hi1 + ui * hr1
                    y1r, y1i = (tr, ti) if y1r is None else (y1r + tr, y1i + ti)
                    if j <= i:
                        hr1, hi1 = ld(NB + i - j, g), ld(NB + i - j, 128 + g)
                        tr = ur * hr1 - ui * hi1
                        ti = ur * hi1 + ui * hr1
                        y0r, y0i = (tr, ti) if y0r is None else (y0r + tr, y0i + ti)
                if sgn > 0:
                    z1r, z1i = y1r - y0i, y1i + y0r
                else:
                    z1r, z1i = y1r + y0i, y1i - y0r
                if i > 0:
                    pr_, pi_ = ld(2 * NB, g), ld(2 * NB, 128 + g)
                    if sgn > 0:
                        y0r, y0i = y0r - pi_, y0i + pr_
                    else:
                        y0r, y0i = y0r + pi_, y0i - pr_
                if i + 2 < NB:
                    spec[zero + 2 * NB, g:g + GR, :] = y1r
                    spec[zero + 2 * NB, 128 + g:128 + g + GR, :] = y1i
                zi = zero + 2 * NB + 1 + i // 2
                h2 = GR // 2
                spec[zi, g // 2:g // 2 + h2, :] = pltpu.bitcast(y0r.astype(BF16), F32)
                spec[zi, 64 + g // 2:64 + g // 2 + h2, :] = pltpu.bitcast(y0i.astype(BF16), F32)
                spec[zi, 128 + g // 2:128 + g // 2 + h2, :] = pltpu.bitcast(z1r.astype(BF16), F32)
                spec[zi, 192 + g // 2:192 + g // 2 + h2, :] = pltpu.bitcast(z1i.astype(BF16), F32)

        def inv(i):
            r0 = (i % 2) * 128
            z = pltpu.bitcast(spec[2 * NB + 1 + i // 2, r0:r0 + 128, :], BF16)
            y = jnp.dot(gmat[...], z, preferred_element_type=F32)
            y = y + kv_load(i).astype(F32) * dv
            ybuf[i * CB:(i + 1) * CB, pl.ds(col, 128)] = y.astype(BF16)

        do_c = "conv" in phases
        do_p = "pre" in phases
        def side(tok):
            if tok[0] == "k" and do_c:
                for j in range(4 * tok[1], 4 * tok[1] + 4):
                    kv_mul(j)
            if tok[0] == "r" and do_p:
                gate[0] = relayout(sl0 + tok[1], tok[1], zero, always, gate[0], RMODE == 'dbl')

        if do_p:
            relayout(sl0, 0, zero, None, None, False)
        if do_c:
            h_dft()
        for tok in SIDE:
            side(tok)
        for su in range(8 * PPI):
            if do_p:
                proj(*_pair_of(c, su // 8), sl0 + su // 8, su // 8, (su // 4) % 2, su % 4)
            if su == DMAPOS:
                prefetch()
            if do_c:
                if su in U_AFTER:
                    for j in range(U_AFTER.index(su) * 4, U_AFTER.index(su) * 4 + 4):
                        u_dft(j)
                for i in INV_AFTER.get(su + 1, ())[:1]:
                    freq_mul(i)
                for i in INV_AFTER.get(su, ()):
                    inv(i)
        return carry

    lax.fori_loop(0, NCH, pro_b, 0)
    for cp in conv_copies(NCH - 1, NCH % 2):
        cp.wait()
    for k in range(PPI):
        wb_copy(NCH, k).wait()
    for n in range(NCH):
        x_copy(n).wait()
        wo_copy(n).wait()

    lhs_q[0:MEM, :] = mem0_ref[...]
    gw = prm[1:2, :]
    scale = DH ** -0.5
    always = jnp.full((8, 128), zsm[0], jnp.int32) == 0

    def combine(b, rows_start, nrows):
        xt = x_v[pl.ds(rows_start, nrows), :].astype(F32)
        g = jax.nn.sigmoid(jnp.sum(xt * gw, axis=-1, keepdims=True))
        a = xt * ybuf[pl.ds(rows_start, nrows), :].astype(F32)
        res = g * a + (1.0 - g) * b
        out_v[pl.ds(rows_start, nrows), :] = res.astype(BF16)
        return res

    def step(s, defer, early, gate, last=False):
        def al(v, n):
            return v if isinstance(v, int) else pl.multiple_of(v, n)

        nride = MEM if last else TPS
        p = al(PM + TPS * s, 8)
        lag = al(TPS * (s - 1) if isinstance(s, int) else jnp.maximum(TPS * (s - 1), 0), 8)
        lhs_q[MEM:MEM + nride, :] = x_v[pl.ds(p, nride), :]
        lhs = [lhs_q[0:MEM + nride, 0:D // 2], lhs_q[0:MEM + nride, D // 2:]]
        cur = al((s % RING) * SEG, SEG)
        offs = [al((p + 8 * k) % (RING * SEG), 8) for k in range(TPS // 8)]
        tok0 = al(s * SEG, SEG)

        def fetch(pr):
            if not last:
                lhs_o[MEM:, pr * 256:(pr + 1) * 256] = obuf[pl.ds(lag, TPS), pr * 256:(pr + 1) * 256]
            nr = TPS if last else SEG
            for tsel in range(3):
                for hh in range(2):
                    t0 = 2 * MEM + hh * SEG
                    cbuf[tsel * 16 + pr, t0:t0 + nr, :] = ring[tsel * H + 2 * pr + hh, pl.ds(cur, nr), :]

        part = {}

        def qkv(pr, tsel, hh, half=None):
            j = tsel * H + 2 * pr + hh
            for hf in ((0, 1) if half is None else (half,)):
                wj = wqkv[2 * _SLOT[(tsel, pr)] + hh, hf * (D // 4):(hf + 1) * (D // 4), :]
                if gate is not None and (pr, tsel, hh, hf) == (GATEPR, 0, 0, 0):
                    wj = jnp.concatenate([jnp.where(always, wj[0:8], gate), wj[8:]], axis=0)
                wj = pltpu.bitcast(wj, BF16)
                t = jnp.dot(lhs[hf], wj, preferred_element_type=F32)
                part[j] = t if hf == 0 else t + part[j]
            if half == 0:
                return
            res = part.pop(j).astype(BF16)
            cbuf[tsel * 16 + pr, hh * MEM:(hh + 1) * MEM, :] = res[0:MEM]
            if last:
                t0 = 2 * MEM + hh * SEG + TPS
                cbuf[tsel * 16 + pr, t0:t0 + MEM, :] = res[MEM:2 * MEM]
                return
            for k in range(TPS // 8):
                ring[j, pl.ds(offs[k], 8), :] = res[MEM + 8 * k:MEM + 8 * (k + 1)]

        probs = {}

        def scores(pr):
            qp = cbuf[pr]
            kp = cbuf[16 + pr]
            sc = lax.dot_general(qp, kp, (((1,), (1,)), ((), ())), preferred_element_type=F32) * scale
            fill = bias[...]
            sc = jnp.where(fill == 0.0, sc, fill)
            mx = jnp.max(sc, axis=-1, keepdims=True)
            e = jnp.exp(sc - mx)
            den = jnp.sum(e, axis=-1, keepdims=True)
            rc = pl.reciprocal(den, approx=True)
            rc = rc * (2.0 - den * rc)
            probs[pr] = (e * rc).astype(BF16)

        def pv(pr, mem_rows=True, tok_rows=True):
            r0 = 0 if mem_rows else 2 * MEM
            r1 = PR if tok_rows else 2 * MEM
            o = jnp.dot(probs[pr][r0:r1], cbuf[32 + pr], preferred_element_type=F32).astype(BF16)
            for hh in range(2):
                c0 = (2 * pr + hh) * DH
                if mem_rows:
                    lhs_o[0:MEM, c0:c0 + DH] = o[hh * MEM:(hh + 1) * MEM]
                if tok_rows:
                    t0 = 2 * MEM + hh * SEG - r0
                    obuf[pl.ds(tok0, SEG), c0:c0 + DH] = o[t0:t0 + SEG]

        accs = [None] * (D // 128)

        def wo(pr, half):
            lo = lhs_o[:, pr * 256:(pr + 1) * 256]
            for nb in range(half * 4, half * 4 + 4):
                wt = pltpu.bitcast(wo_v[nb, pr * 128:(pr + 1) * 128, :], BF16)
                t = jnp.dot(lo, wt, preferred_element_type=F32)
                accs[nb] = t if accs[nb] is None else t + accs[nb]

        NP = H // 2
        late = ()
        main = [("q", pr, t, h) for pr in range(NP) for t in range(3) for h in range(2)]
        if early:
            fetch(0)
            for t in range(3):
                for h in range(2):
                    qkv(0, t, h, 0)
        nt = NP - NDEFER if defer else NP
        main += [("w", pr, hf) for pr in range(nt) for hf in range(2)]
        main += [("w", pr, hf) for hf in range(2) for pr in range(nt, NP)]
        ns = npv = 0
        s_at, pv_at = {}, {}
        for slot, item in enumerate(main):
            if item[0] == "w":
                while item[1] not in pv_at:
                    if npv == ns:
                        scores(ns)
                        s_at[ns] = slot
                        ns += 1
                    pv(npv, tok_rows=npv not in late)
                    pv_at[npv] = slot
                    npv += 1
                if last:
                    tail(slot - 6 * NP)
                else:
                    wo(item[1], item[2])
            else:
                if early and item[1] == 0:
                    qkv(*item[1:], 1)
                else:
                    if item[2] == 0 and item[3] == 0:
                        fetch(item[1])
                    qkv(*item[1:])
            if GROUP == 1:
                if ns < NP and slot + 1 >= 6 * ns + DS:
                    scores(ns)
                    s_at[ns] = slot + 1
                    ns += 1
                if npv < ns and slot + 1 >= s_at[npv] + DPV:
                    pv(npv, tok_rows=npv not in late)
                    pv_at[npv] = slot + 1
                    npv += 1
            elif (slot + 1 - DS) % (6 * GROUP) == 0:
                order = []
                for _ in range(GROUP):
                    if npv < ns and slot + 1 >= s_at[npv] + DPV:
                        order.append(("p", npv))
                        pv_at[npv] = slot + 1
                        npv += 1
                for _ in range(GROUP):
                    if ns < NP and slot + 1 >= 6 * ns + DS:
                        order.append(("s", ns))
                        s_at[ns] = slot + 1
                        ns += 1
                if SFIRST:
                    order = order[::-1]
                for kind, idx in order:
                    if kind == "s":
                        scores(idx)
                    else:
                        pv(idx)
        for pr in late:
            pv(pr, mem_rows=False)
        if last:
            return None
        for nb in range(D // 128):
            lhs_q[0:MEM, nb * 128:(nb + 1) * 128] = accs[nb][0:MEM].astype(BF16)
        acc = jnp.concatenate(accs, axis=1)
        res = combine(acc[MEM:], lag, TPS)
        tk = None
        for r in range(0, TPS, 8):
            for cc in range(0, D, 128):
                t = pltpu.bitcast(res[r:r + 8, cc:cc + 128], U32)
                tk = t if tk is None else tk ^ t
        return tk

    def steps(it, carry):
        s0 = it * UNROLL

        @pl.when(jnp.logical_and(s0 % 8 == OTRIG, s0 > 8))
        def _():
            k = s0 // 8 - 1
            out_copy(pl.multiple_of(k * OCH, OCH), OCH, k).start()

        gate = None
        for u in range(UNROLL):
            gate = step(s0 + u, u + 1 < UNROLL, u > 0, gate if GATEPR >= 0 else None)
        return carry

    nstream = 7
    tail0 = nstream * OCH
    tacc = {}

    def tail(u):
        e, nb = u // 8, u % 8
        a0, na = EPI[e]
        if u == 0:
            out_copy(tail0, EPI[0][0] - tail0, nstream).start()
        tacc[nb] = jnp.dot(obuf[a0:a0 + na, :], pltpu.bitcast(wo_v[nb], BF16), preferred_element_type=F32)
        if nb == 7:
            combine(jnp.concatenate([tacc.pop(n) for n in range(8)], axis=1), a0, na)
            out_copy(a0, na, nstream + 1 + e).start()

    if "main" in phases:
        lax.fori_loop(0, (NSEG - 2) // UNROLL, steps, 0)
    else:
        if "main1" in phases:
            lax.fori_loop(0, 1 + zsm[0], steps, 0)
        if "sink" in phases:
            z = zsm[0]
            out_v[0:16, 0:128] = (ring[z, 0:16, :] + pltpu.bitcast(wqkv[z, 0:8, :], BF16)
                                  + ybuf[pl.ds(pl.multiple_of(z * 16, 16), 16), 0:128])
        for k in range(nstream):
            out_copy(k * OCH, OCH, k).start()
    if "notail" in phases:
        out_copy(tail0, EPI[0][0] - tail0, nstream).start()
        for e, (a0, na) in enumerate(EPI):
            out_copy(a0, na, nstream + 1 + e).start()
    else:
        gate = step(NSEG - 2, True, False, None)
        step(NSEG - 1, False, True, gate if GATEPR >= 0 else None, last=True)

    for k in range(nstream):
        out_copy(k * OCH, OCH, k).wait()
    out_copy(tail0, EPI[0][0] - tail0, nstream).wait()
    for e, (a0, na) in enumerate(EPI):
        out_copy(a0, na, nstream + 1 + e).wait()


def build(phases=("conv", "pre", "main", "epi")):
    @functools.partial(jax.jit, static_argnames=("B_seg_len",))
    def fn(A_q, A_k, A_v, A_shift_k, A_ssm_k, A_ssm_D, B_x, B_mem0, B_Wq, B_Wk, B_Wv, B_Wo,
           B_seg_len, gate_w):
        assert int(B_seg_len) == SEG
        any_spec = pl.BlockSpec(memory_space=pl.ANY)
        vm = pl.BlockSpec(memory_space=pltpu.VMEM)
        out = pl.pallas_call(
            functools.partial(_kernel, phases),
            out_shape=jax.ShapeDtypeStruct((S, D), BF16),
            in_specs=[any_spec] * 8 + [vm] * 4,
            out_specs=any_spec,
            scratch_shapes=[
                pltpu.VMEM((S, D), BF16),
                pltpu.VMEM((PM // 2, D), U32),
                pltpu.VMEM((S, D), BF16),
                pltpu.VMEM((S, D), BF16),
                pltpu.VMEM((3 * H + 2 * PPI, D // 2, DH), U32),
                pltpu.VMEM((2, D // 2, DH), U32),
                pltpu.VMEM((2, D // 2, DH), U32),
                pltpu.VMEM((2, D // 2, DH), U32),
                pltpu.VMEM((2, D // 2, DH), U32),
                pltpu.VMEM((2, D // 2, DH), U32),
                pltpu.VMEM((S // 4, 128), BF16),
                pltpu.VMEM((S // 4, 128), BF16),
                pltpu.VMEM((S // 4, 128), BF16),
                pltpu.VMEM((S // 4, 128), BF16),
                pltpu.VMEM((D // 128, H * DH // 2, 128), U32),
                pltpu.VMEM((3 * H, RING * SEG, DH), BF16),
                pltpu.VMEM((3 * 16, PR, DH), BF16),
                pltpu.VMEM((S, H * DH), BF16),
                pltpu.VMEM((MEM + TPS, D), BF16),
                pltpu.VMEM((MEM + TPS, H * DH), BF16),
                pltpu.VMEM((2, S, 128), BF16),
                pltpu.VMEM((2, S, 128), BF16),
                pltpu.VMEM((2, 128, S), BF16),
                pltpu.VMEM((S + 8, 128), F32),
                pltpu.VMEM((2 * NB + 1 + NB // 2, 256, 128), F32),
                pltpu.VMEM((256, 128), BF16),
                pltpu.VMEM((128, 256), BF16),
                pltpu.VMEM((PR, PR), F32),
                pltpu.VMEM((8, D), F32),
                pltpu.SMEM((1,), jnp.int32),
                pltpu.SemaphoreType.DMA((2, 3)),
                pltpu.SemaphoreType.DMA((2 + NCH,)),
                pltpu.SemaphoreType.DMA((PPA + 2 * PPI, 2)),
                pltpu.SemaphoreType.DMA((8,)),
                pltpu.SemaphoreType.DMA((12,)),
            ],
            compiler_params=pltpu.CompilerParams(vmem_limit_bytes=120 * 1024 * 1024),
        )(A_q.reshape(S, D), A_k.reshape(S, D), A_v.reshape(S, D), A_ssm_k,
          B_Wq.reshape(D // 2, 2, H, DH), B_Wk.reshape(D // 2, 2, H, DH), B_Wv.reshape(D // 2, 2, H, DH),
          B_Wo.reshape(H * DH, D),
          A_shift_k.T, A_ssm_D, gate_w, B_mem0.reshape(MEM, D))
        return out.reshape(1, S, D)
    return fn


pallas_gated_mix__ssm_conv_h3__memory_aug_recurrent_mem_tr__prompt_kernel = build()
```

```python
import math

import jax
import jax.numpy as jnp
from jax import lax
import jax.experimental.pallas as pl
import jax.experimental.pallas.tpu as pltpu

F32 = jnp.float32
BF16 = jnp.bfloat16
U32 = jnp.uint32

S = 2048
D = 1024
H = 32
DH = 128
MEM = 8
SEG = 32
NSEG = S // SEG
NP = H // 2
TPS = 24
PM = S - TPS * (NSEG - 1) - MEM
RING = 18
PR = 2 * (MEM + SEG)
CB = 128
NB = S // CB
NCH = D // 128
GR = 16
PPA = 8
PPI = 5
MSUB = ((0, 144), (144, 128), (272, 128), (400, 128))
XA = MSUB[0][1]
OCH = 192
NSTREAM = 7
EPI = ((1488, 144), (1632, 144), (1776, 144), (1920, 96), (2016, 32))
UNROLL = 2

A_WAIT = {0: (1,), 1: (2,), 2: (3, 4), 4: (5, 6, 7)}
A_START = {0: (("a", 3), ("a", 4)), 1: (("a", 5), ("a", 6), ("a", 7)),
           2: (("c", 0), ("c", 1), ("c", 2), ("b", 0), ("b", 1)), 4: (("b", 2), ("b", 3), ("b", 4))}
U_AFTER = (2, 4, 5, 7)
INV_AFTER = {12: (0, 1), 13: (2, 3), 14: (4, 5), 17: (6, 7), 21: (8, 9), 27: (10, 11), 33: (12, 13),
             39: (14, 15)}
DS = 8
DPV = 9
NDEFER = 6
GATEPR = 2
TAILMIX = 192
TGD = 5


def _pair_of(c, k):
    return ((0, 2 * c), (1, 2 * c), (1, 2 * c + 1), (2, 2 * c), (2, 2 * c + 1))[k]


_SLOT = {(0, 2 * n + 1): n for n in range(PPA)}
_SLOT.update({_pair_of(c, k): PPA + PPI * c + k for c in range(NCH) for k in range(PPI)})


def _dft_matrix(shape, freq_axis):
    r = lax.broadcasted_iota(jnp.int32, shape, freq_axis)
    t = lax.broadcasted_iota(jnp.int32, shape, 1 - freq_axis)
    rr = r & 127
    f = jnp.where(rr < 64, 2 * rr, 2 * (rr - 64) + 1)
    n = ((2 * f + 1) * t + jnp.where(r >= 128, 128, 0)) & 511
    return jnp.cos(n.astype(F32) * (2.0 * math.pi / 512.0))


def _xor_rows(v):
    tk = None
    for r in range(0, v.shape[0], 8):
        for c in range(0, v.shape[1], 128):
            t = pltpu.bitcast(v[r:r + 8, c:c + 128], U32)
            tk = t if tk is None else tk ^ t
    return tk


def _kernel(x_hbm, k_hbm, v_hbm, h_hbm, wq_hbm, wk_hbm, wv_hbm, wo_hbm,
            shift_hbm, dvec_hbm, gw_hbm, mem0_hbm,
            out_hbm,
            x_v, x0, ybuf, out_v, wqkv, kv0, kv1, kv2, kv3, wo_v,
            rg0, rg1, rg2, rg3, rg4, rg5, cbuf, obuf, lhs_q, lhs_o,
            kin, vin, hin, kpad, spec, fmat, gmat, bias, prm,
            shift_ref, dvec_ref, gw_ref, mem0_ref, zsm,
            sem_p, sem_c, sem_x, sem_w, sem_o, sem_out):
    w_u32 = tuple(w.bitcast(U32) for w in (wq_hbm, wk_hbm, wv_hbm))
    wo_u32 = wo_hbm.bitcast(U32)
    kvb = (kv0, kv1, kv2, kv3)
    ring = (rg0, rg1, rg2, rg3, rg4, rg5)

    def conv_copy(c, slot, n):
        if n == 2:
            return pltpu.make_async_copy(h_hbm.at[pl.ds(c * 128, 128), :], hin.at[slot], sem_c.at[slot, 2])
        src, dst = ((k_hbm, kin), (v_hbm, vin))[n]
        return pltpu.make_async_copy(src.at[:, pl.ds(c * 128, 128)], dst.at[slot], sem_c.at[slot, n])

    def w_copies(mat, hp, slot, sem, shared):
        return [pltpu.make_async_copy(
            w_u32[mat].at[:, par, hp, :], wqkv.at[2 * slot + par], sem_w.at[sem, 0 if shared else par])
            for par in range(2)]

    def wa_copies(n):
        return w_copies(0, 2 * n + 1, n, n, False)

    def wb_copies(c, k):
        mat, hp = _pair_of(c, k)
        hp = min(hp, NP - 1) if isinstance(hp, int) else jnp.minimum(hp, NP - 1)
        return w_copies(mat, hp, PPA + PPI * c + k, PPA + c % 2, True)

    def wb_wait(c):
        slabs = wqkv.at[pl.ds(2 * (PPA + PPI * c), 2 * PPI)]
        pltpu.make_async_copy(slabs, slabs, sem_w.at[PPA + c % 2, 0]).wait()

    def wo_copy(n):
        return pltpu.make_async_copy(wo_u32.at[:, pl.ds(n * 128, 128)], wo_v.at[n], sem_o.at[n])

    def x_copy(n):
        r0 = n * (S // NCH)
        rows = pl.ds(r0 if isinstance(n, int) else pl.multiple_of(r0, S // NCH), S // NCH)
        return pltpu.make_async_copy(x_hbm.at[rows, :], x_v.at[rows, :], sem_x.at[2 + n])

    def out_copy(r0, nr, k):
        return pltpu.make_async_copy(out_v.at[pl.ds(r0, nr), :], out_hbm.at[pl.ds(r0, nr), :], sem_out.at[k])

    def x0_copy(part):
        rows = pl.ds(0, XA // 2) if part == 0 else pl.ds(XA // 2, (PM - XA) // 2)
        return pltpu.make_async_copy(x_hbm.bitcast(U32).at[rows, :], x0.at[rows, :], sem_x.at[part])

    def small_copies():
        pairs = ((shift_hbm, shift_ref), (dvec_hbm, dvec_ref), (gw_hbm, gw_ref), (mem0_hbm, mem0_ref))
        return [pltpu.make_async_copy(s_, d_, sem_p.at[n]) for n, (s_, d_) in enumerate(pairs)]

    def start(cps):
        for cp in cps:
            cp.start()

    def wait(cps):
        for cp in cps:
            cp.wait()

    x0_copy(0).start()
    start(wa_copies(0))
    start(small_copies())

    fmat[...] = _dft_matrix((256, 128), 0).astype(BF16)
    x0_copy(1).start()
    start(wa_copies(1))
    gmat[...] = (_dft_matrix((128, 256), 1) * (1.0 / 128.0)).astype(BF16)

    def head_and_pos(idx):
        second = jnp.logical_or(jnp.logical_and(idx >= MEM, idx < 2 * MEM), idx >= 2 * MEM + SEG)
        pos = jnp.where(idx < 2 * MEM, jnp.where(second, idx - MEM, idx),
                        jnp.where(second, idx - MEM - SEG, idx - MEM))
        return second, pos

    qh, ql = head_and_pos(lax.broadcasted_iota(jnp.int32, (PR, PR), 0))
    kh, kl = head_and_pos(lax.broadcasted_iota(jnp.int32, (PR, PR), 1))
    ok = jnp.logical_and(qh == kh, jnp.logical_or(ql < MEM, ql >= kl))
    bias[...] = jnp.where(ok, 0.0, jnp.where(qh == kh, -1e9, -jnp.inf)).astype(F32)

    zsm[0] = 0
    kpad[0:8, :] = jnp.zeros((8, 128), F32)
    obuf[0:TPS, :] = jnp.zeros((TPS, H * DH), BF16)

    def relayout(sl, always=None):
        low = jnp.full((8, DH), 0xFFFF, U32)
        high = jnp.full((8, DH), 0xFFFF0000, U32)
        m = low
        for r0 in range(0, D // 2, 8):
            a = wqkv[2 * sl, r0:r0 + 8, :]
            b = wqkv[2 * sl + 1, r0:r0 + 8, :]
            lo = (a & m) | (b << 16)
            if always is not None:
                hi = (a >> 16) | (b & jnp.where(always, high, lo))
                m = jnp.where(always, low, hi)
            else:
                hi = (a >> 16) | (b & high)
            wqkv[2 * sl, r0:r0 + 8, :] = lo
            wqkv[2 * sl + 1, r0:r0 + 8, :] = hi

    def proj(mat, par, n, sl, hh, ms):
        r0, nr = MSUB[ms]
        res = jnp.dot(pltpu.bitcast(x0[r0 // 2:(r0 + nr) // 2, :], BF16),
                      pltpu.bitcast(wqkv[2 * sl + hh], BF16), preferred_element_type=F32)
        ring[2 * mat + par][2 * n + hh, r0:r0 + nr, :] = res.astype(BF16)

    always = jnp.full((8, 128), zsm[0], jnp.int32) == 0
    x0_copy(0).wait()
    wait(wa_copies(0))
    wait(small_copies())
    start(wa_copies(2))
    prm[0:1, :] = dvec_ref[...].astype(F32).reshape(1, D)
    prm[1:2, :] = gw_ref[...].astype(F32).reshape(1, D)
    relayout(0)
    proj(0, 1, 0, 0, 0, 0)
    proj(0, 1, 0, 0, 1, 0)
    x0_copy(1).wait()
    for n in range(PPA):
        for m_ in A_WAIT.get(n, ()):
            wait(wa_copies(m_))
        for kind, idx in A_START.get(n, ()):
            if kind == "a":
                start(wa_copies(idx))
            elif kind == "b":
                start(wb_copies(0, idx))
            else:
                conv_copy(0, 0, idx).start()
        for su in range(8):
            hh, ms = (su % 2, su // 2) if n == 0 else (su // 4, su % 4)
            if not (n == 0 and ms == 0):
                proj(0, 1, n, n, hh, ms)
            if su == (2 if n == 0 else 0) and n + 1 < PPA:
                relayout(n + 1, always)

    def merged(c, carry):
        slot = c % 2
        wb_wait(c)
        for n in range(3):
            conv_copy(c, slot, n).wait()
        for n in range(3):
            conv_copy(jnp.minimum(c + 1, NCH - 1), 1 - slot, n).start()
        for k in range(PPI):
            start(wb_copies(c + 1, k))
        wo_copy(c).start()
        x_copy(c).start()

        zero = zsm[0]
        always = jnp.full((8, 128), zero, jnp.int32) == 0
        zrow = pl.multiple_of(zero * 16, 16)
        col = pl.multiple_of(c * 128, 128)
        w = shift_ref[:, pl.ds(col, 128)].astype(F32)
        dv = prm[0:1, pl.ds(col, 128)]
        sl0 = PPA + c * PPI
        w3 = jnp.broadcast_to(w[3:4], (8, 128))

        def kv_mul():
            pace = jnp.where(always, w3, pltpu.bitcast(jnp.full((8, DH), 0xFFFF, U32), F32))
            for r0 in range(0, S, 16):
                if r0 and r0 % CB == 0:
                    pace = jnp.where(always, w3, pace)
                kpad[8 + r0:24 + r0, :] = kin[slot, r0:r0 + 16, :].astype(F32)
                vf = vin[slot, r0:r0 + 16, :].astype(F32)
                kvs = []
                for hf in range(2):
                    b0 = 8 + r0 + hf * 8
                    ks = (kpad[b0 - 3:b0 + 5, :] * pace + kpad[b0 - 2:b0 + 6, :] * w[2:3]
                          + kpad[b0 - 1:b0 + 7, :] * w[1:2] + kpad[b0:b0 + 8, :] * w[0:1])
                    kv = ks * vf[hf * 8:(hf + 1) * 8]
                    pace = jnp.where(always, w3, kv)
                    kvs.append(kv)
                kvb[r0 // (4 * CB)][pl.ds(zrow + r0 % (4 * CB), 16), :] = (
                    jnp.concatenate(kvs, axis=0).astype(BF16))

        def kv_load(j):
            return kvb[j // 4][(j % 4) * CB:(j % 4 + 1) * CB, :]

        def ld(idx, r0):
            return spec[idx, r0:r0 + GR, :]

        def freq_mul(i):
            for g in range(0, 128, GR):
                even = g < 64
                hr, hi = ld(NB + i + 1, g), ld(NB + i + 1, 128 + g)
                y0r = y0i = y1r = y1i = None
                for j in range(i + 2):
                    ur, ui = ld(j, g), ld(j, 128 + g)
                    tr = ur * hr - ui * hi
                    ti = ur * hi + ui * hr
                    y1r, y1i = (tr, ti) if y1r is None else (y1r + tr, y1i + ti)
                    if j <= i:
                        hr, hi = ld(NB + i - j, g), ld(NB + i - j, 128 + g)
                        tr = ur * hr - ui * hi
                        ti = ur * hi + ui * hr
                        y0r, y0i = (tr, ti) if y0r is None else (y0r + tr, y0i + ti)
                z1r, z1i = (y1r - y0i, y1i + y0r) if even else (y1r + y0i, y1i - y0r)
                if i > 0:
                    pr_, pi_ = ld(2 * NB, g), ld(2 * NB, 128 + g)
                    y0r, y0i = (y0r - pi_, y0i + pr_) if even else (y0r + pi_, y0i - pr_)
                if i + 2 < NB:
                    spec[zero + 2 * NB, g:g + GR, :] = y1r
                    spec[zero + 2 * NB, 128 + g:128 + g + GR, :] = y1i
                zi = zero + 2 * NB + 1 + i // 2
                for q, val in enumerate((y0r, y0i, z1r, z1i)):
                    r0 = 64 * q + g // 2
                    spec[zi, r0:r0 + GR // 2, :] = pltpu.bitcast(val.astype(BF16), F32)

        def inv(i):
            r0 = (i % 2) * 128
            z = pltpu.bitcast(spec[2 * NB + 1 + i // 2, r0:r0 + 128, :], BF16)
            y = jnp.dot(gmat[...], z, preferred_element_type=F32)
            y = y + kv_load(i).astype(F32) * dv
            ybuf[i * CB:(i + 1) * CB, pl.ds(col, 128)] = y.astype(BF16)

        relayout(sl0)
        for m_ in range(NB):
            spec[zero + NB + m_] = lax.dot_general(
                fmat[...], hin[slot, :, m_ * CB:(m_ + 1) * CB], (((1,), (1,)), ((), ())),
                preferred_element_type=F32)
        for k in range(1, PPI):
            relayout(sl0 + k)
        kv_mul()
        for su in range(8 * PPI):
            mat, par = _pair_of(0, su // 8)
            proj(mat, par, c, sl0 + su // 8, (su // 4) % 2, su % 4)
            if su in U_AFTER:
                for j in range(U_AFTER.index(su) * 4, U_AFTER.index(su) * 4 + 4):
                    spec[zero + j] = jnp.dot(fmat[...], kv_load(j), preferred_element_type=F32)
            for i in INV_AFTER.get(su + 1, ())[:1]:
                freq_mul(i)
            for i in INV_AFTER.get(su, ()):
                inv(i)
        return carry

    lax.fori_loop(0, NCH, merged, 0)
    for n in range(3):
        conv_copy(NCH - 1, NCH % 2, n).wait()
    wb_wait(NCH)
    for n in range(NCH):
        x_copy(n).wait()
        wo_copy(n).wait()

    lhs_q[0:MEM, :] = mem0_ref[...]
    gw = prm[1:2, :]
    scale = DH ** -0.5
    always = jnp.full((8, 128), zsm[0], jnp.int32) == 0

    def gated(wt, tok):
        return jnp.concatenate([jnp.where(always, wt[0:8], tok), wt[8:]], axis=0)

    tpos = [0]
    tacc, tgate, tg = {}, {}, {}

    def tail():
        u = tpos[0]
        tpos[0] += 1
        e, nb, kg = u // 64, (u // 8) % 8, u % 8
        a0, na = EPI[e]
        if u == 0:
            out_copy(NSTREAM * OCH, EPI[0][0] - NSTREAM * OCH, NSTREAM).start()
        wt = wo_v[nb, kg * 256:(kg + 1) * 256, :]
        if u in tgate:
            wt = gated(wt, tgate.pop(u))
        t = jnp.dot(obuf[a0:a0 + na, kg * 512:(kg + 1) * 512], pltpu.bitcast(wt, BF16),
                    preferred_element_type=F32)
        tacc[nb] = t if kg == 0 else t + tacc[nb]
        if nb == 0 and kg == 0:
            xt = x_v[a0:a0 + na, :].astype(F32)
            tg[e] = jax.nn.sigmoid(jnp.sum(xt * gw, axis=-1, keepdims=True))
        if kg == 7:
            cols = slice(nb * 128, (nb + 1) * 128)
            g = tg[e]
            a = x_v[a0:a0 + na, cols].astype(F32) * ybuf[a0:a0 + na, cols].astype(F32)
            res = g * a + (1.0 - g) * tacc.pop(nb)
            out_v[a0:a0 + na, cols] = res.astype(BF16)
            tgate[u + TGD] = _xor_rows(res)
            if nb == 7:
                out_copy(a0, na, NSTREAM + 1 + e).start()

    def step(s, chained_next, chained_prev, gate, last=False):
        def al(v, n):
            return v if isinstance(v, int) else pl.multiple_of(v, n)

        nride = MEM if last else TPS
        p = al(PM + TPS * s, 8)
        lag = al(TPS * (s - 1) if isinstance(s, int) else jnp.maximum(TPS * (s - 1), 0), 8)
        lhs_q[MEM:MEM + nride, :] = x_v[pl.ds(p, nride), :]
        lhs = [lhs_q[0:MEM + nride, 0:D // 2], lhs_q[0:MEM + nride, D // 2:]]
        cur = al((s % RING) * SEG, SEG)
        offs = [al((p + 8 * k) % (RING * SEG), 8) for k in range(TPS // 8)]
        tok0 = al(s * SEG, SEG)

        def fetch(pr):
            if not last:
                lhs_o[MEM:, pr * 256:(pr + 1) * 256] = obuf[pl.ds(lag, TPS), pr * 256:(pr + 1) * 256]
            nr = TPS if last else SEG
            for mat in range(3):
                for hh in range(2):
                    t0 = 2 * MEM + hh * SEG
                    cbuf[mat * NP + pr, t0:t0 + nr, :] = (
                        ring[2 * mat + pr % 2][2 * (pr // 2) + hh, pl.ds(cur, nr), :])

        part = {}

        def qkv(pr, mat, hh, half=None):
            for hf in ((0, 1) if half is None else (half,)):
                wj = wqkv[2 * _SLOT[(mat, pr)] + hh, hf * (D // 4):(hf + 1) * (D // 4), :]
                if gate is not None and (pr, mat, hh, hf) == (GATEPR, 0, 0, 0):
                    wj = gated(wj, gate)
                t = jnp.dot(lhs[hf], pltpu.bitcast(wj, BF16), preferred_element_type=F32)
                part[mat, hh] = t if hf == 0 else t + part[mat, hh]
                if last and tpos[0] < TAILMIX:
                    tail()
            if half == 0:
                return
            res = part.pop((mat, hh)).astype(BF16)
            cbuf[mat * NP + pr, hh * MEM:(hh + 1) * MEM, :] = res[0:MEM]
            if last:
                t0 = 2 * MEM + hh * SEG + TPS
                cbuf[mat * NP + pr, t0:t0 + MEM, :] = res[MEM:2 * MEM]
                return
            for k in range(TPS // 8):
                ring[2 * mat + pr % 2][2 * (pr // 2) + hh, pl.ds(offs[k], 8), :] = (
                    res[MEM + 8 * k:MEM + 8 * (k + 1)])

        probs = {}

        def scores(pr):
            sc = lax.dot_general(cbuf[pr], cbuf[NP + pr], (((1,), (1,)), ((), ())),
                                 preferred_element_type=F32) * scale
            fill = bias[...]
            sc = jnp.where(fill == 0.0, sc, fill)
            mx = jnp.max(sc, axis=-1, keepdims=True)
            e = jnp.exp(sc - mx)
            den = jnp.sum(e, axis=-1, keepdims=True)
            rc = pl.reciprocal(den, approx=True)
            rc = rc * (2.0 - den * rc)
            probs[pr] = (e * rc).astype(BF16)

        def pv(pr):
            o = jnp.dot(probs.pop(pr), cbuf[2 * NP + pr], preferred_element_type=F32).astype(BF16)
            for hh in range(2):
                c0 = (2 * pr + hh) * DH
                lhs_o[0:MEM, c0:c0 + DH] = o[hh * MEM:(hh + 1) * MEM]
                t0 = 2 * MEM + hh * SEG
                obuf[pl.ds(tok0, SEG), c0:c0 + DH] = o[t0:t0 + SEG]

        accs = [None] * (D // 128)

        def wo(pr, half):
            lo = lhs_o[:, pr * 256:(pr + 1) * 256]
            for nb in range(half * 4, half * 4 + 4):
                wt = pltpu.bitcast(wo_v[nb, pr * 128:(pr + 1) * 128, :], BF16)
                t = jnp.dot(lo, wt, preferred_element_type=F32)
                accs[nb] = t if accs[nb] is None else t + accs[nb]

        order = [("q", pr, mat, hh) for pr in range(NP) for mat in range(3) for hh in range(2)]
        nt = NP - NDEFER if chained_next else NP
        order += [("w", pr, hf) for pr in range(nt) for hf in range(2)]
        order += [("w", pr, hf) for hf in range(2) for pr in range(nt, NP)]
        if chained_prev:
            fetch(0)
            for mat in range(3):
                for hh in range(2):
                    qkv(0, mat, hh, 0)
        ns = npv = 0
        s_at = {}
        for slot, item in enumerate(order):
            if item[0] == "w":
                assert item[1] < npv
                if last:
                    tail()
                else:
                    wo(item[1], item[2])
            elif chained_prev and item[1] == 0:
                qkv(*item[1:], 1)
            else:
                if item[2] == 0 and item[3] == 0:
                    fetch(item[1])
                qkv(*item[1:])
            if ns < NP and slot + 1 >= 6 * ns + DS:
                scores(ns)
                s_at[ns] = slot + 1
                ns += 1
            if npv < ns and slot + 1 >= s_at[npv] + DPV:
                pv(npv)
                npv += 1
        if last:
            while tpos[0] < 64 * len(EPI):
                tail()
            return None
        for nb in range(D // 128):
            lhs_q[0:MEM, nb * 128:(nb + 1) * 128] = accs[nb][0:MEM].astype(BF16)
        b = jnp.concatenate(accs, axis=1)[MEM:]
        xt = x_v[pl.ds(lag, TPS), :].astype(F32)
        g = jax.nn.sigmoid(jnp.sum(xt * gw, axis=-1, keepdims=True))
        a = xt * ybuf[pl.ds(lag, TPS), :].astype(F32)
        res = g * a + (1.0 - g) * b
        out_v[pl.ds(lag, TPS), :] = res.astype(BF16)
        return _xor_rows(res) if chained_next else None

    def steps(it, carry):
        s0 = it * UNROLL

        @pl.when(jnp.logical_and(s0 % 8 == UNROLL, s0 > 8))
        def _():
            k = s0 // 8 - 1
            out_copy(pl.multiple_of(k * OCH, OCH), OCH, k).start()

        gate = None
        for u in range(UNROLL):
            gate = step(s0 + u, u + 1 < UNROLL, u > 0, gate)
        return carry

    lax.fori_loop(0, NSEG // UNROLL - 1, steps, 0)
    gate = None
    for s in range(NSEG - UNROLL, NSEG):
        gate = step(s, s + 1 < NSEG, s > NSEG - UNROLL, gate, last=s + 1 == NSEG)

    for k in range(NSTREAM):
        out_copy(k * OCH, OCH, k).wait()
    out_copy(NSTREAM * OCH, EPI[0][0] - NSTREAM * OCH, NSTREAM).wait()
    for e, (a0, na) in enumerate(EPI):
        out_copy(a0, na, NSTREAM + 1 + e).wait()


@jax.jit
def pallas_gated_mix__ssm_conv_h3__memory_aug_recurrent_mem_tr__prompt_kernel(
    A_q: jax.Array,
    A_k: jax.Array,
    A_v: jax.Array,
    A_shift_k: jax.Array,
    A_ssm_k: jax.Array,
    A_ssm_D: jax.Array,
    B_x: jax.Array,
    B_mem0: jax.Array,
    B_Wq: jax.Array,
    B_Wk: jax.Array,
    B_Wv: jax.Array,
    B_Wo: jax.Array,
    B_seg_len: jax.Array,
    gate_w: jax.Array,
):
    del B_x, B_seg_len
    any_spec = pl.BlockSpec(memory_space=pl.ANY)
    out = pl.pallas_call(
        _kernel,
        out_shape=jax.ShapeDtypeStruct((S, D), BF16),
        in_specs=[any_spec] * 12,
        out_specs=any_spec,
        scratch_shapes=[
            pltpu.VMEM((S, D), BF16),
            pltpu.VMEM((PM // 2, D), U32),
            pltpu.VMEM((S, D), BF16),
            pltpu.VMEM((S, D), BF16),
            pltpu.VMEM((3 * H + 2 * PPI, D // 2, DH), U32),
        ] + [pltpu.VMEM((S // 4, 128), BF16)] * 4 + [
            pltpu.VMEM((D // 128, H * DH // 2, 128), U32),
        ] + [pltpu.VMEM((NP, RING * SEG, DH), BF16)] * 6 + [
            pltpu.VMEM((3 * NP, PR, DH), BF16),
            pltpu.VMEM((S, H * DH), BF16),
            pltpu.VMEM((MEM + TPS, D), BF16),
            pltpu.VMEM((MEM + TPS, H * DH), BF16),
            pltpu.VMEM((2, S, 128), BF16),
            pltpu.VMEM((2, S, 128), BF16),
            pltpu.VMEM((2, 128, S), BF16),
            pltpu.VMEM((S + 8, 128), F32),
            pltpu.VMEM((2 * NB + 1 + NB // 2, 256, 128), F32),
            pltpu.VMEM((256, 128), BF16),
            pltpu.VMEM((128, 256), BF16),
            pltpu.VMEM((PR, PR), F32),
            pltpu.VMEM((8, D), F32),
            pltpu.VMEM((4, D), BF16),
            pltpu.VMEM((D,), BF16),
            pltpu.VMEM((D,), BF16),
            pltpu.VMEM((MEM, D), BF16),
            pltpu.SMEM((1,), jnp.int32),
            pltpu.SemaphoreType.DMA((4,)),
            pltpu.SemaphoreType.DMA((2, 3)),
            pltpu.SemaphoreType.DMA((2 + NCH,)),
            pltpu.SemaphoreType.DMA((PPA + 2, 2)),
            pltpu.SemaphoreType.DMA((NCH,)),
            pltpu.SemaphoreType.DMA((NSTREAM + 1 + len(EPI),)),
        ],
        compiler_params=pltpu.CompilerParams(vmem_limit_bytes=120 * 1024 * 1024,
                                             disable_bounds_checks=True),
    )(A_q.reshape(S, D), A_k.reshape(S, D), A_v.reshape(S, D), A_ssm_k,
      B_Wq.reshape(D // 2, 2, H, DH), B_Wk.reshape(D // 2, 2, H, DH), B_Wv.reshape(D // 2, 2, H, DH),
      B_Wo.reshape(H * DH, D),
      A_shift_k.T, A_ssm_D, gate_w, B_mem0.reshape(MEM, D))
    return out.reshape(1, S, D)
```

```python
import math

import jax
import jax.numpy as jnp
from jax import lax
import jax.experimental.pallas as pl
import jax.experimental.pallas.tpu as pltpu

F32 = jnp.float32
BF16 = jnp.bfloat16
U32 = jnp.uint32

S = 2048
D = 1024
H = 32
DH = 128
MEM = 8
SEG = 32
NSEG = S // SEG
NP = H // 2
TPS = 24
PM = S - TPS * (NSEG - 1) - MEM
RING = 18
PR = 2 * (MEM + SEG)
CB = 128
NB = S // CB
NCH = D // 128
GR = 16
PPA = 8
PPI = 5
MSUB = ((0, 144), (144, 128), (272, 128), (400, 128))
OCH = 192
NSTREAM = 7
EPI = ((1488, 144), (1632, 144), (1776, 144), (1920, 96), (2016, 32))
UNROLL = 3
NFIRST = 3

ALL = (0, 1, 2, 3)
PLAN_A = (
    ("start", ("x", 0), ("a", 0), ("p",)), ("const", "f"), ("start", ("x", 1), ("x", 2)),
    ("wait", ("x", 0), ("a", 0)), ("start", ("x", 3), ("a", 1)),
    ("relayout", 0, False), ("proj", 0, (0,)),
    ("wait", ("x", 1), ("x", 2)), ("start", ("a", 2)),
    ("proj", 0, (1, 2)),
    ("wait", ("x", 3), ("a", 1), ("p",)), ("start", ("a", 3), ("a", 4)),
    ("relayout", 1, False), ("proj", 0, (3,)), ("proj", 1, (0, 1)),
    ("wait", ("a", 2)), ("start", ("a", 5), ("a", 6), ("a", 7)),
    ("relayout", 2, True), ("proj", 1, (2, 3)), ("proj", 2, (0, 1)),
    ("wait", ("a", 3), ("a", 4)), ("start", ("c", 0), ("c", 1), ("c", 2)),
    ("relayout", 3, True), ("proj", 2, (2, 3)), ("const", "rest"), ("const", "g"),
    ("relayout", 4, True), ("proj", 3, ALL), ("proj", 4, (0, 1)),
    ("wait", ("a", 5), ("a", 6), ("a", 7)), ("start", ("b", 0), ("b", 1), ("b", 2), ("b", 3), ("b", 4)),
    ("relayout", 5, True), ("proj", 4, (2, 3)), ("relayout", 6, True), ("proj", 5, ALL),
    ("relayout", 7, True), ("proj", 6, ALL), ("proj", 7, ALL),
)
U_AFTER = (2, 4, 5, 7)
INV_AFTER = {12: (0, 1), 13: (2, 3), 14: (4, 5), 17: (6, 7), 21: (8, 9), 27: (10, 11), 33: (12, 13),
             39: (14, 15)}
DS = 11
DPV = 10
NDEFER = 4
GATEPR = 1
TAILMIX = 192
TGD = 10


def _pair_of(c, k):
    return ((0, 2 * c), (1, 2 * c), (1, 2 * c + 1), (2, 2 * c), (2, 2 * c + 1))[k]


_SLOT = {(0, 2 * n + 1): n for n in range(PPA)}
_SLOT.update({_pair_of(c, k): PPA + PPI * c + k for c in range(NCH) for k in range(PPI)})


def _dft_matrix():
    r = lax.broadcasted_iota(jnp.int32, (256, CB), 0)
    t = lax.broadcasted_iota(jnp.int32, (256, CB), 1)
    rr = r & 127
    f = jnp.where(rr < 64, 2 * rr, 2 * (rr - 64) + 1)
    n = ((2 * f + 1) * t + jnp.where(r >= 128, 128, 0)) & 511
    return jnp.cos(n.astype(F32) * (2.0 * math.pi / 512.0))


def _xor_rows(v):
    tk = None
    for r in range(0, v.shape[0], 8):
        for c in range(0, v.shape[1], 128):
            t = pltpu.bitcast(v[r:r + 8, c:c + 128], U32)
            tk = t if tk is None else tk ^ t
    return tk


def _kernel(x_hbm, k_hbm, v_hbm, h_hbm, wq_hbm, wk_hbm, wv_hbm, wo_hbm,
            shift_hbm, dvec_hbm, gw_hbm, mem0_hbm,
            out_hbm,
            x_v, x0, ybuf, out_v, wqkv, kv0, kv1, kv2, kv3, wo_v,
            rg0, rg1, rg2, rg3, rg4, rg5, cbuf, obuf, lhs_q, lhs_o,
            kin, vin, hin, kpad, spec, fmat, gmat, bias, prm,
            shift_ref, dvec_ref, gw_ref, mem0_ref, zsm,
            sem_p, sem_c, sem_x, sem_w, sem_o, sem_out):
    w_u32 = tuple(w.bitcast(U32) for w in (wq_hbm, wk_hbm, wv_hbm))
    wo_u32 = wo_hbm.bitcast(U32)
    kvb = (kv0, kv1, kv2, kv3)
    ring = (rg0, rg1, rg2, rg3, rg4, rg5)

    def conv_copy(c, slot, n):
        if n == 2:
            return pltpu.make_async_copy(h_hbm.at[pl.ds(c * 128, 128), :], hin.at[slot], sem_c.at[slot, 2])
        src, dst = ((k_hbm, kin), (v_hbm, vin))[n]
        return pltpu.make_async_copy(src.at[:, pl.ds(c * 128, 128)], dst.at[slot], sem_c.at[slot, n])

    def w_copies(mat, hp, slot, sem, shared):
        return [pltpu.make_async_copy(
            w_u32[mat].at[:, par, hp, :], wqkv.at[2 * slot + par], sem_w.at[sem, 0 if shared else par])
            for par in range(2)]

    def wa_copies(n):
        return w_copies(0, 2 * n + 1, n, n, False)

    def wb_copies(c, k):
        mat, hp = _pair_of(c, k)
        hp = min(hp, NP - 1) if isinstance(hp, int) else jnp.minimum(hp, NP - 1)
        return w_copies(mat, hp, PPA + PPI * c + k, PPA + (c & 1), True)

    def wb_wait(c):
        slabs = wqkv.at[pl.ds(2 * (PPA + PPI * c), 2 * PPI)]
        pltpu.make_async_copy(slabs, slabs, sem_w.at[PPA + (c & 1), 0]).wait()

    def wo_copy(n):
        return pltpu.make_async_copy(wo_u32.at[:, pl.ds(n * 128, 128)], wo_v.at[n], sem_o.at[n])

    def x_copy(n):
        r0 = n * (S // NCH)
        rows = pl.ds(r0 if isinstance(n, int) else pl.multiple_of(r0, S // NCH), S // NCH)
        return pltpu.make_async_copy(x_hbm.at[rows, :], x_v.at[rows, :], sem_x.at[4 + n])

    def out_copy(r0, nr, k):
        return pltpu.make_async_copy(out_v.at[pl.ds(r0, nr), :], out_hbm.at[pl.ds(r0, nr), :], sem_out.at[k])

    def x0_copy(part):
        rows = pl.ds(MSUB[part][0] // 2, MSUB[part][1] // 2)
        return pltpu.make_async_copy(x_hbm.bitcast(U32).at[rows, :], x0.at[rows, :], sem_x.at[part])

    def small_copies():
        pairs = ((shift_hbm, shift_ref), (dvec_hbm, dvec_ref), (gw_hbm, gw_ref), (mem0_hbm, mem0_ref))
        return [pltpu.make_async_copy(s_, d_, sem_p.at[n]) for n, (s_, d_) in enumerate(pairs)]

    def start(cps):
        for cp in cps:
            cp.start()

    def wait(cps):
        for cp in cps:
            cp.wait()

    def copies(kind, idx=None):
        if kind == "x":
            return [x0_copy(idx)]
        if kind == "a":
            return wa_copies(idx)
        if kind == "b":
            return wb_copies(0, idx)
        if kind == "c":
            return [conv_copy(0, 0, idx)]
        return small_copies()

    def const_f():
        fmat[...] = _dft_matrix().astype(BF16)

    def const_g():
        gmat[...] = (fmat[...].astype(F32).T * (1.0 / 128.0)).astype(BF16)

    def head_and_pos(idx):
        second = jnp.logical_or(jnp.logical_and(idx >= MEM, idx < 2 * MEM), idx >= 2 * MEM + SEG)
        pos = jnp.where(idx < 2 * MEM, jnp.where(second, idx - MEM, idx),
                        jnp.where(second, idx - MEM - SEG, idx - MEM))
        return second, pos

    def const_rest():
        qh, ql = head_and_pos(lax.broadcasted_iota(jnp.int32, (PR, PR), 0))
        kh, kl = head_and_pos(lax.broadcasted_iota(jnp.int32, (PR, PR), 1))
        ok = jnp.logical_and(qh == kh, jnp.logical_or(ql < MEM, ql >= kl))
        bias[...] = jnp.where(ok, 0.0, jnp.where(qh == kh, -1e9, -jnp.inf)).astype(F32)
        kpad[0:8, :] = jnp.zeros((8, 128), F32)
        lhs_o[MEM:2 * MEM, :] = jnp.zeros((MEM, H * DH), BF16)
        prm[0:1, :] = dvec_ref[...].astype(F32).reshape(1, D)
        prm[1:2, :] = gw_ref[...].astype(F32).reshape(1, D)

    zsm[0] = 0

    def relayout(sl, always=None):
        low = jnp.full((8, DH), 0xFFFF, U32)
        high = jnp.full((8, DH), 0xFFFF0000, U32)
        m = low
        for r0 in range(0, D // 2, 8):
            a = wqkv[2 * sl, r0:r0 + 8, :]
            b = wqkv[2 * sl + 1, r0:r0 + 8, :]
            lo = (a & m) | (b << 16)
            if always is not None:
                hi = (a >> 16) | (b & jnp.where(always, high, lo))
                m = jnp.where(always, low, hi)
            else:
                hi = (a >> 16) | (b & high)
            wqkv[2 * sl, r0:r0 + 8, :] = lo
            wqkv[2 * sl + 1, r0:r0 + 8, :] = hi

    def proj(mat, par, n, sl, hh, ms):
        r0, nr = MSUB[ms]
        res = jnp.dot(pltpu.bitcast(x0[r0 // 2:(r0 + nr) // 2, :], BF16),
                      pltpu.bitcast(wqkv[2 * sl + hh], BF16), preferred_element_type=F32)
        ring[2 * mat + par][2 * n + hh, r0:r0 + nr, :] = res.astype(BF16)

    always = jnp.full((8, 128), zsm[0], jnp.int32) == 0
    for op in PLAN_A:
        if op[0] == "start":
            for item in op[1:]:
                start(copies(*item))
        elif op[0] == "wait":
            for item in op[1:]:
                wait(copies(*item))
        elif op[0] == "const":
            {"f": const_f, "g": const_g, "rest": const_rest}[op[1]]()
        elif op[0] == "relayout":
            relayout(op[1], always if op[2] else None)
        else:
            for hh, ms in ([(h_, m_) for m_ in op[2] for h_ in range(2)] if len(op[2]) < 4 else
                           [(h_, m_) for h_ in range(2) for m_ in op[2]]):
                proj(0, 1, op[1], op[1], hh, ms)

    def merged(c, carry):
        slot = c & 1
        wb_wait(c)
        for n in range(3):
            conv_copy(c, slot, n).wait()
        for n in (2, 0, 1):
            conv_copy(jnp.minimum(c + 1, NCH - 1), 1 - slot, n).start()
        for k in range(PPI):
            start(wb_copies(c + 1, k))
        wo_copy(c).start()
        x_copy(c).start()

        zero = zsm[0]
        always = jnp.full((8, 128), zero, jnp.int32) == 0
        zrow = pl.multiple_of(zero * 16, 16)
        col = pl.multiple_of(c * 128, 128)
        w = shift_ref[:, pl.ds(col, 128)].astype(F32)
        dv = prm[0:1, pl.ds(col, 128)]
        sl0 = PPA + c * PPI
        w3 = jnp.broadcast_to(w[3:4], (8, 128))

        def kv_mul():
            pace = w3
            for r0 in range(0, S, 16):
                kpad[8 + r0:24 + r0, :] = kin[slot, r0:r0 + 16, :].astype(F32)
                vf = vin[slot, r0:r0 + 16, :].astype(F32)
                kvs = []
                for hf in range(2):
                    b0 = 8 + r0 + hf * 8
                    ks = (kpad[b0 - 3:b0 + 5, :] * pace + kpad[b0 - 2:b0 + 6, :] * w[2:3]
                          + kpad[b0 - 1:b0 + 7, :] * w[1:2] + kpad[b0:b0 + 8, :] * w[0:1])
                    kv = ks * vf[hf * 8:(hf + 1) * 8]
                    pace = jnp.where(always, w3, kv)
                    kvs.append(kv)
                kvb[r0 // (4 * CB)][pl.ds(zrow + r0 % (4 * CB), 16), :] = (
                    jnp.concatenate(kvs, axis=0).astype(BF16))

        def kv_load(j):
            return kvb[j // 4][(j % 4) * CB:(j % 4 + 1) * CB, :]

        def ld(idx, r0):
            return spec[idx, r0:r0 + GR, :]

        def freq_mul(i):
            for g in range(0, 128, GR):
                even = g < 64
                hr, hi = ld(NB + i + 1, g), ld(NB + i + 1, 128 + g)
                y0r = y0i = y1r = y1i = None
                for j in range(i + 2):
                    ur, ui = ld(j, g), ld(j, 128 + g)
                    tr = ur * hr - ui * hi
                    ti = ur * hi + ui * hr
                    y1r, y1i = (tr, ti) if y1r is None else (y1r + tr, y1i + ti)
                    if j <= i:
                        hr, hi = ld(NB + i - j, g), ld(NB + i - j, 128 + g)
                        tr = ur * hr - ui * hi
                        ti = ur * hi + ui * hr
                        y0r, y0i = (tr, ti) if y0r is None else (y0r + tr, y0i + ti)
                z1r, z1i = (y1r - y0i, y1i + y0r) if even else (y1r + y0i, y1i - y0r)
                if i > 0:
                    pr_, pi_ = ld(2 * NB, g), ld(2 * NB, 128 + g)
                    y0r, y0i = (y0r - pi_, y0i + pr_) if even else (y0r + pi_, y0i - pr_)
                if i + 2 < NB:
                    spec[zero + 2 * NB, g:g + GR, :] = y1r
                    spec[zero + 2 * NB, 128 + g:128 + g + GR, :] = y1i
                zi = zero + 2 * NB + 1 + i // 2
                for q, val in enumerate((y0r, y0i, z1r, z1i)):
                    r0 = 64 * q + g // 2
                    spec[zi, r0:r0 + GR // 2, :] = pltpu.bitcast(val.astype(BF16), F32)

        def inv(i):
            r0 = (i % 2) * 128
            z = pltpu.bitcast(spec[2 * NB + 1 + i // 2, r0:r0 + 128, :], BF16)
            y = jnp.dot(gmat[...], z, preferred_element_type=F32)
            y = y + kv_load(i).astype(F32) * dv
            ybuf[i * CB:(i + 1) * CB, pl.ds(col, 128)] = y.astype(BF16)

        relayout(sl0)
        for m_ in range(NB):
            spec[zero + NB + m_] = lax.dot_general(
                fmat[...], hin[slot, :, m_ * CB:(m_ + 1) * CB], (((1,), (1,)), ((), ())),
                preferred_element_type=F32)
        for k in range(1, PPI):
            relayout(sl0 + k)
        kv_mul()
        for su in range(8 * PPI):
            mat, par = _pair_of(0, su // 8)
            if not (mat == 2 and su % 4 == 3):
                proj(mat, par, c, sl0 + su // 8, (su // 4) % 2, su % 4)
            if su in U_AFTER:
                for j in range(U_AFTER.index(su) * 4, U_AFTER.index(su) * 4 + 4):
                    spec[zero + j] = jnp.dot(fmat[...], kv_load(j), preferred_element_type=F32)
            for i in INV_AFTER.get(su + 1, ())[:1]:
                freq_mul(i)
            for i in INV_AFTER.get(su, ()):
                inv(i)
        return carry

    lax.fori_loop(0, NCH, merged, 0)
    for n in range(3):
        conv_copy(NCH - 1, NCH % 2, n).wait()
    wb_wait(NCH)
    for n in range(NCH):
        x_copy(n).wait()
        wo_copy(n).wait()

    lhs_q[0:MEM, :] = mem0_ref[...]
    gw = prm[1:2, :]
    scale = DH ** -0.5
    always = jnp.full((8, 128), zsm[0], jnp.int32) == 0

    def gated(wt, tok):
        return jnp.concatenate([jnp.where(always, wt[0:8], tok), wt[8:]], axis=0)

    lpos = [0]
    lacc = [None]

    def late():
        u = lpos[0]
        lpos[0] += 1
        pr, hh, hf = u // 4, (u // 2) % 2, u % 2
        r0, nr = MSUB[3]
        wj = wqkv[2 * _SLOT[(2, pr)] + hh, hf * (D // 4):(hf + 1) * (D // 4), :]
        t = jnp.dot(pltpu.bitcast(x0[r0 // 2:(r0 + nr) // 2, hf * (D // 2):(hf + 1) * (D // 2)], BF16),
                    pltpu.bitcast(wj, BF16), preferred_element_type=F32)
        lacc[0] = t if hf == 0 else t + lacc[0]
        if hf == 1:
            ring[4 + pr % 2][2 * (pr // 2) + hh, r0:r0 + nr, :] = lacc[0].astype(BF16)

    tpos = [0]
    tacc, tgate, tg = {}, {}, {}

    def tail():
        u = tpos[0]
        tpos[0] += 1
        e, nb, kg = u // 64, (u // 8) % 8, u % 8
        a0, na = EPI[e]
        if u == 0:
            out_copy(NSTREAM * OCH, EPI[0][0] - NSTREAM * OCH, NSTREAM).start()
        wt = wo_v[nb, kg * 256:(kg + 1) * 256, :]
        if u in tgate:
            wt = gated(wt, tgate.pop(u))
        t = jnp.dot(obuf[a0:a0 + na, kg * 512:(kg + 1) * 512], pltpu.bitcast(wt, BF16),
                    preferred_element_type=F32)
        tacc[nb] = t if kg == 0 else t + tacc[nb]
        if nb == 0 and kg == 0:
            xt = x_v[a0:a0 + na, :].astype(F32)
            tg[e] = jax.nn.sigmoid(jnp.sum(xt * gw, axis=-1, keepdims=True))
        if kg == 7:
            cols = slice(nb * 128, (nb + 1) * 128)
            g = tg[e]
            a = x_v[a0:a0 + na, cols].astype(F32) * ybuf[a0:a0 + na, cols].astype(F32)
            res = g * a + (1.0 - g) * tacc.pop(nb)
            out_v[a0:a0 + na, cols] = res.astype(BF16)
            tgate[u + TGD] = _xor_rows(res)
            if nb == 7:
                out_copy(a0, na, NSTREAM + 1 + e).start()

    def step(s, chained_next, chained_prev, gate):
        def al(v, n):
            return v if isinstance(v, int) else pl.multiple_of(v, n)

        first = isinstance(s, int) and s == 0
        last = isinstance(s, int) and s == NSEG - 1

        nride = MEM if last else TPS
        p = al(PM + TPS * s, 8)
        lag = al(TPS * (s - 1), 8)
        lhs_q[MEM:MEM + nride, :] = x_v[pl.ds(p, nride), :]
        lhs = [lhs_q[0:MEM + nride, 0:D // 2], lhs_q[0:MEM + nride, D // 2:]]
        cur = al((s % RING) * SEG, SEG)
        offs = [al((p + 8 * k) % (RING * SEG), 8) for k in range(TPS // 8)]
        tok0 = al(s * SEG, SEG)

        def fetch(pr):
            if not (first or last):
                lhs_o[MEM:, pr * 256:(pr + 1) * 256] = obuf[pl.ds(lag, TPS), pr * 256:(pr + 1) * 256]
            nr = TPS if last else SEG
            for mat in range(3):
                for hh in range(2):
                    t0 = 2 * MEM + hh * SEG
                    cbuf[mat * NP + pr, t0:t0 + nr, :] = (
                        ring[2 * mat + pr % 2][2 * (pr // 2) + hh, pl.ds(cur, nr), :])

        part = {}

        def qkv(pr, mat, hh, half=None):
            for hf in ((0, 1) if half is None else (half,)):
                wj = wqkv[2 * _SLOT[(mat, pr)] + hh, hf * (D // 4):(hf + 1) * (D // 4), :]
                if gate is not None and (pr, mat, hh, hf) == (GATEPR, 0, 0, 0):
                    wj = gated(wj, gate)
                t = jnp.dot(lhs[hf], pltpu.bitcast(wj, BF16), preferred_element_type=F32)
                part[mat, hh] = t if hf == 0 else t + part[mat, hh]
                if last and tpos[0] < TAILMIX:
                    tail()
            if half == 0:
                return
            res = part.pop((mat, hh)).astype(BF16)
            cbuf[mat * NP + pr, hh * MEM:(hh + 1) * MEM, :] = res[0:MEM]
            if last:
                t0 = 2 * MEM + hh * SEG + TPS
                cbuf[mat * NP + pr, t0:t0 + MEM, :] = res[MEM:2 * MEM]
                return
            for k in range(TPS // 8):
                ring[2 * mat + pr % 2][2 * (pr // 2) + hh, pl.ds(offs[k], 8), :] = (
                    res[MEM + 8 * k:MEM + 8 * (k + 1)])

        probs = {}

        def scores(pr):
            sc = lax.dot_general(cbuf[pr], cbuf[NP + pr], (((1,), (1,)), ((), ())),
                                 preferred_element_type=F32) * scale
            fill = bias[...]
            sc = jnp.where(fill == 0.0, sc, fill)
            mx = jnp.max(sc, axis=-1, keepdims=True)
            e = jnp.exp(sc - mx)
            den = jnp.sum(e, axis=-1, keepdims=True)
            rc = pl.reciprocal(den, approx=True)
            rc = rc * (2.0 - den * rc)
            probs[pr] = (e * rc).astype(BF16)

        def pv(pr):
            o = jnp.dot(probs.pop(pr), cbuf[2 * NP + pr], preferred_element_type=F32).astype(BF16)
            for hh in range(2):
                c0 = (2 * pr + hh) * DH
                lhs_o[0:MEM, c0:c0 + DH] = o[hh * MEM:(hh + 1) * MEM]
                t0 = 2 * MEM + hh * SEG
                obuf[pl.ds(tok0, SEG), c0:c0 + DH] = o[t0:t0 + SEG]

        accs = [None] * (D // 128)

        def wo(pr, half):
            lo = lhs_o[0:2 * MEM if first else MEM + TPS, pr * 256:(pr + 1) * 256]
            for nb in range(half * 4, half * 4 + 4):
                wt = pltpu.bitcast(wo_v[nb, pr * 128:(pr + 1) * 128, :], BF16)
                t = jnp.dot(lo, wt, preferred_element_type=F32)
                accs[nb] = t if accs[nb] is None else t + accs[nb]
                if first and nb % 2 == 1:
                    late()

        order = [("q", pr, mat, hh) for pr in range(NP) for mat in range(3) for hh in range(2)]
        nt = NP - NDEFER if chained_next else NP
        order += [("w", pr, hf) for pr in range(nt) for hf in range(2)]
        order += [("w", pr, hf) for hf in range(2) for pr in range(nt, NP)]
        if chained_prev:
            fetch(0)
            for mat in range(3):
                for hh in range(2):
                    qkv(0, mat, hh, 0)
        if last and not chained_prev:
            tail()
        ns = npv = 0
        s_at = {}
        for slot, item in enumerate(order):
            if item[0] == "w":
                while item[1] >= npv:
                    if npv == ns:
                        scores(ns)
                        s_at[ns] = slot
                        ns += 1
                    pv(npv)
                    npv += 1
                if last:
                    tail()
                else:
                    wo(item[1], item[2])
            elif chained_prev and item[1] == 0:
                qkv(*item[1:], 1)
            else:
                if item[2] == 0 and item[3] == 0:
                    fetch(item[1])
                qkv(*item[1:])
            if (slot + 1 - DS) % 12 == 0:
                do_pv = [n for n in (npv, npv + 1) if n < ns and slot + 1 >= s_at[n] + DPV]
                do_s = [n for n in (ns, ns + 1) if n < NP and slot + 1 >= 6 * n + DS]
                for n in do_s[::-1]:
                    scores(n)
                    s_at[n] = slot + 1
                for n in do_pv[::-1]:
                    pv(n)
                ns += len(do_s)
                npv += len(do_pv)
        if last:
            while tpos[0] < 64 * len(EPI):
                tail()
            return None
        for nb in range(D // 128):
            lhs_q[0:MEM, nb * 128:(nb + 1) * 128] = accs[nb][0:MEM].astype(BF16)
        if first:
            return None
        b = jnp.concatenate(accs, axis=1)[MEM:]
        xt = x_v[pl.ds(lag, TPS), :].astype(F32)
        g = jax.nn.sigmoid(jnp.sum(xt * gw, axis=-1, keepdims=True))
        a = xt * ybuf[pl.ds(lag, TPS), :].astype(F32)
        res = g * a + (1.0 - g) * b
        out_v[pl.ds(lag, TPS), :] = res.astype(BF16)
        return _xor_rows(res) if chained_next else None

    def steps(it, carry):
        s0 = NFIRST + it * UNROLL

        @pl.when(jnp.logical_and((s0 - 1) % 8 < UNROLL, s0 > 8))
        def _():
            k = (s0 - 1) // 8 - 1
            out_copy(pl.multiple_of(k * OCH, OCH), OCH, k).start()

        gate = None
        for u in range(UNROLL):
            gate = step(s0 + u, u + 1 < UNROLL, u > 0, gate)
        return carry

    gate = None
    for s in range(NFIRST):
        gate = step(s, s + 1 < NFIRST, s > 0, gate)
    nloop = (NSEG - 1 - NFIRST) // UNROLL
    lax.fori_loop(0, nloop, steps, 0)
    rest = NFIRST + nloop * UNROLL
    started = [(s0 - 1) // 8 - 1 for s0 in range(NFIRST, rest, UNROLL) if (s0 - 1) % 8 < UNROLL and s0 > 8]
    assert started == list(range(len(started))) and NSTREAM * OCH <= TPS * (rest - 1)
    for k in range(len(started), NSTREAM):
        out_copy(k * OCH, OCH, k).start()
    gate = None
    for s in range(rest, NSEG):
        gate = step(s, s + 1 < NSEG, s > rest, gate)

    for k in range(NSTREAM):
        out_copy(k * OCH, OCH, k).wait()
    out_copy(NSTREAM * OCH, EPI[0][0] - NSTREAM * OCH, NSTREAM).wait()
    for e, (a0, na) in enumerate(EPI):
        out_copy(a0, na, NSTREAM + 1 + e).wait()


@jax.jit
def pallas_gated_mix__ssm_conv_h3__memory_aug_recurrent_mem_tr__prompt_kernel(
    A_q: jax.Array,
    A_k: jax.Array,
    A_v: jax.Array,
    A_shift_k: jax.Array,
    A_ssm_k: jax.Array,
    A_ssm_D: jax.Array,
    B_x: jax.Array,
    B_mem0: jax.Array,
    B_Wq: jax.Array,
    B_Wk: jax.Array,
    B_Wv: jax.Array,
    B_Wo: jax.Array,
    B_seg_len: jax.Array,
    gate_w: jax.Array,
):
    del B_x, B_seg_len
    any_spec = pl.BlockSpec(memory_space=pl.ANY)
    out = pl.pallas_call(
        _kernel,
        out_shape=jax.ShapeDtypeStruct((S, D), BF16),
        in_specs=[any_spec] * 12,
        out_specs=any_spec,
        scratch_shapes=[
            pltpu.VMEM((S, D), BF16),
            pltpu.VMEM((PM // 2, D), U32),
            pltpu.VMEM((S, D), BF16),
            pltpu.VMEM((S, D), BF16),
            pltpu.VMEM((3 * H + 2 * PPI, D // 2, DH), U32),
        ] + [pltpu.VMEM((S // 4, 128), BF16)] * 4 + [
            pltpu.VMEM((D // 128, H * DH // 2, 128), U32),
        ] + [pltpu.VMEM((NP, RING * SEG, DH), BF16)] * 6 + [
            pltpu.VMEM((3 * NP, PR, DH), BF16),
            pltpu.VMEM((S, H * DH), BF16),
            pltpu.VMEM((MEM + TPS, D), BF16),
            pltpu.VMEM((MEM + TPS, H * DH), BF16),
            pltpu.VMEM((2, S, 128), BF16),
            pltpu.VMEM((2, S, 128), BF16),
            pltpu.VMEM((2, 128, S), BF16),
            pltpu.VMEM((S + 8, 128), F32),
            pltpu.VMEM((2 * NB + 1 + NB // 2, 256, 128), F32),
            pltpu.VMEM((256, 128), BF16),
            pltpu.VMEM((128, 256), BF16),
            pltpu.VMEM((PR, PR), F32),
            pltpu.VMEM((8, D), F32),
            pltpu.VMEM((4, D), BF16),
            pltpu.VMEM((D,), BF16),
            pltpu.VMEM((D,), BF16),
            pltpu.VMEM((MEM, D), BF16),
            pltpu.SMEM((1,), jnp.int32),
            pltpu.SemaphoreType.DMA((4,)),
            pltpu.SemaphoreType.DMA((2, 3)),
            pltpu.SemaphoreType.DMA((4 + NCH,)),
            pltpu.SemaphoreType.DMA((PPA + 2, 2)),
            pltpu.SemaphoreType.DMA((NCH,)),
            pltpu.SemaphoreType.DMA((NSTREAM + 1 + len(EPI),)),
        ],
        compiler_params=pltpu.CompilerParams(vmem_limit_bytes=120 * 1024 * 1024,
                                             disable_bounds_checks=True),
    )(A_q.reshape(S, D), A_k.reshape(S, D), A_v.reshape(S, D), A_ssm_k,
      B_Wq.reshape(D // 2, 2, H, DH), B_Wk.reshape(D // 2, 2, H, DH), B_Wv.reshape(D // 2, 2, H, DH),
      B_Wo.reshape(H * DH, D),
      A_shift_k.T, A_ssm_D, gate_w, B_mem0.reshape(MEM, D))
    return out.reshape(1, S, D)
```
